```python
import os as _os
_os.environ.setdefault("JAX_PLATFORMS", "cpu")
import jax
import jax.numpy as jnp

def _softmax(x, axis=-1):
    return jax.nn.softmax(x, axis=axis)
def _gelu(x):
    return jax.nn.gelu(x, approximate=True)
def _silu(x):
    return jax.nn.silu(x)
def _sigmoid(x):
    return jax.nn.sigmoid(x)
def _layernorm(x, axis=-1, eps=1e-5):
    m = jnp.mean(x, axis=axis, keepdims=True)
    v = jnp.var(x, axis=axis, keepdims=True)
    return (x - m) / jnp.sqrt(v + eps)
def _scatter_add(tgt, idx, src, axis=0):
    return tgt.at[idx].add(src)
def _segment_sum(src, seg, n):
    return jax.ops.segment_sum(src, seg, n)
class _Rng:
    def __init__(self, key):
        self._k = key
    def _next(self):
        self._k, sub = jax.random.split(self._k)
        return sub
    def normal(self, shape):
        return jax.random.normal(self._next(), shape, dtype=jnp.bfloat16)
    def randint(self, lo, hi, shape):
        return jax.random.randint(self._next(), shape, lo, hi, dtype=jnp.int32)
    def uniform(self, shape, lo=0.0, hi=1.0):
        return jax.random.uniform(self._next(), shape, jnp.bfloat16, lo, hi)
    def permutation(self, n):
        return jax.random.permutation(self._next(), n)


kernel_name = 'gated_mix__mha_block_cached__gqa_block_cached__decode'

def setup_inputs():
    _rng = _Rng(jax.random.key(int.from_bytes(__import__("os").urandom(4), "little")))
    _w = (lambda a: (lambda t: t.astype(jnp.bfloat16) if jnp.issubdtype(t.dtype, jnp.floating) else t)(jnp.asarray(a)))
    def _A_setup():
        B, Sq, D = 4, 1, 512
        H, Sk, Dh = 32, 8192, 128
        return {
            "x": _w((lambda *s: _rng.normal(s) * 0.05)(B, Sq, D)),
            "k_cache": _w((lambda *s: _rng.normal(s) * 3.2)(B, H, Sk, Dh)),
            "v_cache": _w((lambda *s: _rng.normal(s) * 0.05)(B, H, Sk, Dh)),
            "wq": _w((lambda *s: _rng.normal(s) * 3.2)(D, H * Dh) * (D ** -0.5)),
            "wo": _w((lambda *s: _rng.normal(s) * 0.05)(H * Dh, D) * ((H * Dh) ** -0.5)),
        }
    _A_in = _A_setup()

    def _B_setup():
        B, Sq, D = 4, 1, 512
        Hq, Hkv, Sk, Dh = 32, 8, 8192, 128
        assert Hq % Hkv == 0, (Hq, Hkv)
        return {
            "x": _w((lambda *s: _rng.normal(s) * 0.05)(B, Sq, D)),
            "k_cache": _w((lambda *s: _rng.normal(s) * 3.2)(B, Hkv, Sk, Dh)),
            "v_cache": _w((lambda *s: _rng.normal(s) * 0.05)(B, Hkv, Sk, Dh)),
            "wq": _w((lambda *s: _rng.normal(s) * 3.2)(D, Hq * Dh) * (D ** -0.5)),
            "wo": _w((lambda *s: _rng.normal(s) * 0.05)(Hq * Dh, D) * ((Hq * Dh) ** -0.5)),
        }
    _B_in = _B_setup()

    return {
        "A_x": _A_in["x"],
        "A_k_cache": _A_in["k_cache"],
        "A_v_cache": _A_in["v_cache"],
        "A_wq": _A_in["wq"],
        "A_wo": _A_in["wo"],
        "B_x": _B_in["x"],
        "B_k_cache": _B_in["k_cache"],
        "B_v_cache": _B_in["v_cache"],
        "B_wq": _B_in["wq"],
        "B_wo": _B_in["wo"],
        "gate_w": _w((lambda *s: _rng.normal(s) * 0.05)(512) * 16.0),
    }

def reference(A_x, A_k_cache, A_v_cache, A_wq, A_wo, B_x, B_k_cache, B_v_cache, B_wq, B_wo, gate_w):
    def _A_ref(x, k_cache, v_cache, wq, wo):
        B, Sq, D = x.shape
        H, Dh = 32, 128
        q = (lambda x, *d: x.transpose(*d))((x @ wq).reshape(B, Sq, H, Dh), 0, 2, 1, 3)
        scores = jnp.einsum("bhqd,bhkd->bhqk", q, k_cache) * (Dh ** -0.5)
        p = _softmax(scores, axis=-1)
        o = jnp.einsum("bhqk,bhkd->bhqd", p, v_cache)
        return (lambda x, *d: x.transpose(*d))(o, 0, 2, 1, 3).reshape(B, Sq, H * Dh) @ wo

    def _B_ref(x, k_cache, v_cache, wq, wo):
        B, Sq, D = x.shape
        Hq, Dh = 32, 128
        Hkv = k_cache.shape[1]
        rep = Hq // Hkv
        q = (lambda x, *d: x.transpose(*d))((x @ wq).reshape(B, Sq, Hq, Dh), 0, 2, 1, 3)
        k = jnp.repeat(k_cache, rep, axis=1)
        v = jnp.repeat(v_cache, rep, axis=1)
        scores = jnp.einsum("bhqd,bhkd->bhqk", q, k) * (Dh ** -0.5)
        p = _softmax(scores, axis=-1)
        o = jnp.einsum("bhqk,bhkd->bhqd", p, v)
        return (lambda x, *d: x.transpose(*d))(o, 0, 2, 1, 3).reshape(B, Sq, Hq * Dh) @ wo

    x = A_x
    g = _sigmoid((x * gate_w).sum(-1, keepdims=True))
    a = _A_ref(x, A_k_cache, A_v_cache, A_wq, A_wo)
    b = _B_ref(x, B_k_cache, B_v_cache, B_wq, B_wo)
    return g * a + (1 - g) * b
```

```python
import functools
import jax
import jax.numpy as jnp
from jax import lax
from jax.experimental import pallas as pl
from jax.experimental.pallas import tpu as pltpu

NB = 4
D = 512
H = 32
HKV = 8
S = 8192
DH = 128
NGA = NB * H
NGB = NB * HKV
NG = NGA + NGB
REP = H // HKV


def split(start, n, R):
    out = []
    while n > 0:
        r = min(R, n)
        out.append((start, r)); start += r; n -= r
    return out


def _make_kernel(CH=2048, R=128, mode="half", rot=0, dbg=None, WA0=8, WAN=16):
    NCH = S // CH
    scale = DH ** -0.5
    f32 = jnp.float32
    bf16 = jnp.bfloat16

    if mode == "half":
        h = CH // 2
        pk = []
        for a, b in zip(split(0, h, R), split(h, h, R)):
            pk += [a + (0,), b + (1,)]
        pv = pk
    elif mode == "kv":
        pk = [a + (0,) for a in split(0, CH, R)]
        vs = split(0, CH, R)
        vs = vs[rot:] + vs[:rot]
        pv = [a + (1,) for a in vs]
    else:
        raise ValueError(mode)

    def kernel(xa_hbm, ka_hbm, va_hbm, wqa_hbm, woa_hbm, kb_hbm, vb_hbm, wqb_hbm, wob_hbm, gw_hbm,
               out_ref,
               kbuf, vbuf, wqa_buf, wqb_buf, woa_buf, wob_buf, xa_buf, gw_buf,
               xa_tab, ga_tab, gb_tab, acc_ref,
               kv_sem, wqb_sem, wob_sem, wa_sem, s_sem):

        def start_arr(src, buf, pat, which, grp, j):
            if dbg == 'nodma':
                return
            for r0, n, th in pat:
                pltpu.make_async_copy(src.at[grp, pl.ds(j * CH + r0, n), :],
                                      buf.at[j, pl.ds(r0, n), :], kv_sem.at[which, j]).start(priority=th)

        def start_k(k_hbm, grp, j):
            start_arr(k_hbm, kbuf, pk, 0, grp, j)

        def start_v(v_hbm, grp, j):
            start_arr(v_hbm, vbuf, pv, 1, grp, j)

        def wait_k(j):
            if dbg == 'nodma':
                return
            pltpu.make_async_copy(kbuf.at[j], kbuf.at[j], kv_sem.at[0, j]).wait()

        def wait_v(j):
            if dbg == 'nodma':
                return
            pltpu.make_async_copy(vbuf.at[j], vbuf.at[j], kv_sem.at[1, j]).wait()

        def start_wq_head(src, buf, h, sem, t0=0):
            for r in range(D // 128):
                pltpu.make_async_copy(src.at[pl.ds(r * 128, 128), pl.ds(pl.multiple_of(h * DH, DH), DH)],
                                      buf.at[h, pl.ds(r * 128, 128), :], sem).start(priority=(r + t0) % 2)

        def start_wo_head(src, buf, h, sem, t0=0):
            for r in range(DH // 32):
                row = pl.multiple_of(h * DH + r * 32, 32)
                pltpu.make_async_copy(src.at[pl.ds(row, 32), :],
                                      buf.at[pl.ds(row, 32), :], sem).start(priority=(r + t0) % 2)

        def start_wqb(hk):
            for r in range(REP):
                start_wq_head(wqb_hbm, wqb_buf, hk * REP + r, wqb_sem.at[hk])

        def start_wob(hk):
            for r in range(REP):
                start_wo_head(wob_hbm, wob_buf, hk * REP + r, wob_sem.at[hk])

        def wait_wqb(hk):
            v = wqb_buf.at[pl.ds(hk * REP, REP)]
            pltpu.make_async_copy(v, v, wqb_sem.at[hk]).wait()

        def wait_wob(hk):
            v = wob_buf.at[pl.ds(pl.multiple_of(hk * REP * DH, REP * DH), REP * DH)]
            pltpu.make_async_copy(v, v, wob_sem.at[hk]).wait()

        cxa = pltpu.make_async_copy(xa_hbm, xa_buf, s_sem.at[0])
        cgw = pltpu.make_async_copy(gw_hbm, gw_buf, s_sem.at[1])
        cxa.start(); cgw.start()
        start_wqb(0)
        start_k(kb_hbm, 0, 0)
        start_v(vb_hbm, 0, 0)
        start_wob(0)
        for j in range(1, NCH):
            start_k(kb_hbm, 0, j)
            start_v(vb_hbm, 0, j)

        cxa.wait(); cgw.wait()
        xa = xa_buf[...].astype(f32)
        gw = gw_buf[...].astype(f32).reshape(1, D)
        gate = jax.nn.sigmoid(jnp.sum(xa * gw, axis=1, keepdims=True))
        for b in range(NB):
            xa_tab[b] = jnp.broadcast_to(xa[b:b + 1, :], (8, D))
        gate8 = jnp.concatenate([gate, jnp.zeros((8 - NB, 1), f32)], axis=0)
        ga_tab[...] = jnp.broadcast_to(gate8, (8, D))
        gb_tab[...] = jnp.broadcast_to(1.0 - gate8, (8, D))
        acc_ref[...] = jnp.zeros_like(acc_ref)

        row_d = lax.broadcasted_iota(jnp.int32, (8, D), 0)
        row_h = lax.broadcasted_iota(jnp.int32, (8, DH), 0) % REP

        def attend(q, g, next_src):
            m = l = acc = None
            for j in range(NCH):
                wait_k(j)
                s = lax.dot_general(q, kbuf[j], (((1,), (1,)), ((), ())), preferred_element_type=f32) * scale
                next_src(0, j)
                m_c = jnp.max(s, axis=1, keepdims=True)
                m_new = m_c if j == 0 else jnp.maximum(m, m_c)
                p = jnp.exp(s - m_new)
                l_c = jnp.sum(p, axis=1, keepdims=True)
                wait_v(j)
                pv_ = jnp.dot(p.astype(bf16), vbuf[j], preferred_element_type=f32)
                next_src(1, j)
                if j == 0:
                    l, acc = l_c, pv_
                else:
                    alpha = jnp.exp(m - m_new)
                    l = alpha * l + l_c
                    acc = alpha * acc + pv_
                m = m_new
            return (acc / l)

        def group_b(g, carry):
            b = g // HKV
            hk = g % HKV

            @pl.when(g < HKV)
            def _():
                @pl.when(g + 1 < HKV)
                def _():
                    start_wqb(g + 1)
                    start_wob(g + 1)
                wait_wqb(g)

            @pl.when(jnp.logical_and(g >= WA0, g < WA0 + WAN))
            def _():
                per = H // WAN
                for r in range(per):
                    h = (g - WA0) * per + r
                    start_wq_head(wqa_hbm, wqa_buf, h, wa_sem.at[0])
                    start_wo_head(woa_hbm, woa_buf, h, wa_sem.at[1])

            x = xa_tab[b].astype(bf16)
            q = None
            for r in range(REP):
                qr = jnp.dot(x, wqb_buf[hk * REP + r], preferred_element_type=f32)
                q = qr if r == 0 else jnp.where(row_h == r, qr, q)
            q = q.astype(bf16)

            def nxt(which, j):
                @pl.when(g + 1 < NGB)
                def _():
                    (start_k, start_v)[which]((kb_hbm, vb_hbm)[which], g + 1, j)

                @pl.when(g + 1 == NGB)
                def _():
                    (start_k, start_v)[which]((ka_hbm, va_hbm)[which], 0, j)

            o = attend(q, g, nxt)
            o = o.astype(bf16).astype(f32)

            @pl.when(g < HKV)
            def _():
                wait_wob(g)

            lhs = jnp.concatenate([jnp.broadcast_to(o[r:r + 1, :], (8, DH)) for r in range(REP)], axis=1)
            w = wob_buf[pl.ds(pl.multiple_of(hk * REP * DH, REP * DH), REP * DH), :]
            res = jnp.dot(lhs.astype(bf16), w, preferred_element_type=f32)
            acc_ref[...] += jnp.where(row_d == b, res * gb_tab[...], 0.0)
            return carry

        lax.fori_loop(0, NGB, group_b, 0)

        pltpu.make_async_copy(wqa_buf, wqa_buf, wa_sem.at[0]).wait()
        pltpu.make_async_copy(woa_buf, woa_buf, wa_sem.at[1]).wait()

        def group_a(g, carry):
            b = g // H
            h = g % H
            x = xa_tab[b].astype(bf16)
            q = jnp.dot(x, wqa_buf[h], preferred_element_type=f32).astype(bf16)

            def nxt(which, j):
                @pl.when(g + 1 < NGA)
                def _():
                    (start_k, start_v)[which]((ka_hbm, va_hbm)[which], g + 1, j)

            o = attend(q, g, nxt).astype(bf16)
            w = woa_buf[pl.ds(pl.multiple_of(h * DH, DH), DH), :]
            res = jnp.dot(o, w, preferred_element_type=f32)
            acc_ref[...] += jnp.where(row_d == b, res * ga_tab[...], 0.0)
            return carry

        lax.fori_loop(0, NGA, group_a, 0)

        out_ref[...] = acc_ref[0:NB, :].astype(out_ref.dtype)

    scratch = [
        pltpu.VMEM((NCH, CH, DH), bf16),
        pltpu.VMEM((NCH, CH, DH), bf16),
        pltpu.VMEM((H, D, DH), bf16),
        pltpu.VMEM((H, D, DH), bf16),
        pltpu.VMEM((H * DH, D), bf16),
        pltpu.VMEM((H * DH, D), bf16),
        pltpu.VMEM((NB, D), bf16),
        pltpu.VMEM((D,), bf16),
        pltpu.VMEM((NB, 8, D), f32),
        pltpu.VMEM((8, D), f32),
        pltpu.VMEM((8, D), f32),
        pltpu.VMEM((8, D), f32),
        pltpu.SemaphoreType.DMA((2, NCH)),
        pltpu.SemaphoreType.DMA((HKV,)),
        pltpu.SemaphoreType.DMA((HKV,)),
        pltpu.SemaphoreType.DMA((2,)),
        pltpu.SemaphoreType.DMA((2,)),
    ]

    def run(A_x, A_k_cache, A_v_cache, A_wq, A_wo, B_x, B_k_cache, B_v_cache, B_wq, B_wo, gate_w):
        ka = A_k_cache.reshape(NGA, S, DH)
        va = A_v_cache.reshape(NGA, S, DH)
        kb = B_k_cache.reshape(NGB, S, DH)
        vb = B_v_cache.reshape(NGB, S, DH)
        any_spec = pl.BlockSpec(memory_space=pl.ANY)
        return pl.pallas_call(
            kernel,
            out_shape=jax.ShapeDtypeStruct((NB, D), bf16),
            in_specs=[any_spec] * 10,
            out_specs=pl.BlockSpec(memory_space=pltpu.VMEM),
            scratch_shapes=scratch,
            compiler_params=pltpu.CompilerParams(vmem_limit_bytes=100 * 1024 * 1024, disable_bounds_checks=True),
        )(A_x.reshape(NB, D), ka, va, A_wq, A_wo, kb, vb, B_wq, B_wo, gate_w).reshape(NB, 1, D)
    return run


_run = _make_kernel(R=160)


@jax.jit
def pallas_gated_mix__mha_block_cached__gqa_block_cached__decode_kernel(
    A_x, A_k_cache, A_v_cache, A_wq, A_wo, B_x, B_k_cache, B_v_cache, B_wq, B_wo, gate_w,
):
    return _run(A_x, A_k_cache, A_v_cache, A_wq, A_wo, B_x, B_k_cache, B_v_cache, B_wq, B_wo, gate_w)
```

```python
import functools
import jax
import jax.numpy as jnp
from jax import lax
from jax.experimental import pallas as pl
from jax.experimental.pallas import tpu as pltpu

NB = 4
D = 512
H = 32
HKV = 8
S = 8192
DH = 128
NGA = NB * H
NGB = NB * HKV
REP = H // HKV


def split(start, n, R):
    out = []
    while n > 0:
        r = min(R, n)
        out.append((start, r)); start += r; n -= r
    return out


def _make_kernel(CH=2048, NS=6, R=192, rot=0, dbg=None, WA0=8, WAN=16, swap=False):
    NCH = S // CH
    NCA = NGA * NCH
    NCB = NGB * NCH
    scale = DH ** -0.5
    f32 = jnp.float32
    bf16 = jnp.bfloat16

    ks = split(0, CH, R)
    vs = split(0, CH, R)
    vs = vs[rot:] + vs[:rot]
    TK, TV = (1, 0) if swap else (0, 1)

    def kernel(xa_hbm, ka_hbm, va_hbm, wqa_hbm, woa_hbm, kb_hbm, vb_hbm, wqb_hbm, wob_hbm, gw_hbm,
               out_ref,
               kbuf, vbuf, wqa_buf, wqb_buf, woa_buf, wob_buf, xa_buf, gw_buf,
               q_tab, ga_tab, gb_tab, acc_ref,
               kv_sem, w_sem, s_sem):

        def slot_of(cg):
            return cg % NS if isinstance(cg, int) else lax.rem(cg, NS)

        def kv_copy(src, c, buf, which, slot, r0, n):
            row = c * CH + r0
            if not isinstance(row, int):
                row = pl.multiple_of(row, 16)
            return pltpu.make_async_copy(src.at[pl.ds(row, n), :],
                                         buf.at[slot, pl.ds(r0, n), :], kv_sem.at[which, slot])

        def start_pair(k_src, kc, kslot, v_src, vc, vslot):
            if dbg == 'nodma':
                return
            for (kr, kn), (vr, vn) in zip(ks, vs):
                kv_copy(k_src, kc, kbuf, 0, kslot, kr, kn).start(priority=TK)
                kv_copy(v_src, vc, vbuf, 1, vslot, vr, vn).start(priority=TV)

        def start_alone(src, c, buf, which, slot):
            if dbg == 'nodma':
                return
            for i, (r0, n) in enumerate(ks):
                kv_copy(src, c, buf, which, slot, r0, n).start(priority=i % 2)

        def wait_k(slot):
            if dbg == 'nodma':
                return
            pltpu.make_async_copy(kbuf.at[slot], kbuf.at[slot], kv_sem.at[0, slot]).wait()

        def wait_v(slot):
            if dbg == 'nodma':
                return
            pltpu.make_async_copy(vbuf.at[slot], vbuf.at[slot], kv_sem.at[1, slot]).wait()

        def start_wq_piece(src, buf, rblk, sem):
            row = rblk * 16
            if not isinstance(row, int):
                row = pl.multiple_of(row, 16)
            for c in range(4):
                pltpu.make_async_copy(src.at[pl.ds(row, 16), pl.ds(c * 1024, 1024)],
                                      buf.at[pl.ds(row, 16), pl.ds(c * 1024, 1024)], sem).start(priority=c % 2)

        def start_wo_piece(src, buf, rblk, sem):
            for r in range(4):
                row = rblk * 128 + r * 32
                if not isinstance(row, int):
                    row = pl.multiple_of(row, 32)
                pltpu.make_async_copy(src.at[pl.ds(row, 32), :],
                                      buf.at[pl.ds(row, 32), :], sem).start(priority=r % 2)

        def wait_all(buf, sem):
            pltpu.make_async_copy(buf, buf, sem).wait()

        cxa = pltpu.make_async_copy(xa_hbm, xa_buf, s_sem.at[0])
        cgw = pltpu.make_async_copy(gw_hbm, gw_buf, s_sem.at[1])
        cxa.start(); cgw.start()
        for i in range(32):
            start_wq_piece(wqb_hbm, wqb_buf, i, w_sem.at[0])
        start_alone(kb_hbm, 0, kbuf, 0, 0)
        for c in range(1, NS):
            start_pair(kb_hbm, c, c, vb_hbm, c - 1, c - 1)
        for i in range(32):
            start_wo_piece(wob_hbm, wob_buf, i, w_sem.at[1])

        cxa.wait(); cgw.wait()
        xa = xa_buf[...].astype(f32)
        gw = gw_buf[...].astype(f32).reshape(1, D)
        gate = jax.nn.sigmoid(jnp.sum(xa * gw, axis=1, keepdims=True))
        x8 = jnp.concatenate([xa, jnp.zeros((8 - NB, D), f32)], axis=0).astype(bf16)

        def fill_q_tab(wq_buf):
            q_all = jnp.dot(x8, wq_buf[...], preferred_element_type=f32)
            for h in range(H):
                q_tab[h] = q_all[:, h * DH:(h + 1) * DH]

        gate8 = jnp.concatenate([gate, jnp.zeros((8 - NB, 1), f32)], axis=0)
        ga_tab[...] = jnp.broadcast_to(gate8, (8, D))
        gb_tab[...] = jnp.broadcast_to(1.0 - gate8, (8, D))
        acc_ref[...] = jnp.zeros_like(acc_ref)

        row_d = lax.broadcasted_iota(jnp.int32, (8, D), 0)
        row_h = lax.broadcasted_iota(jnp.int32, (8, DH), 0) % REP

        def attend(q, cg0, next_src):
            m = l = acc = None
            for j in range(NCH):
                slot = slot_of(cg0 + j)
                wait_k(slot)
                s = lax.dot_general(q, kbuf[slot], (((1,), (1,)), ((), ())), preferred_element_type=f32) * scale
                next_src(j, slot, slot_of(cg0 + j + NS - 1))
                m_c = jnp.max(s, axis=1, keepdims=True)
                m_new = m_c if j == 0 else jnp.maximum(m, m_c)
                p = jnp.exp(s - m_new)
                l_c = jnp.sum(p, axis=1, keepdims=True)
                wait_v(slot)
                pv_ = jnp.dot(p.astype(bf16), vbuf[slot], preferred_element_type=f32)
                if j == 0:
                    l, acc = l_c, pv_
                else:
                    alpha = jnp.exp(m - m_new)
                    l = alpha * l + l_c
                    acc = alpha * acc + pv_
                m = m_new
            return (acc / l)

        def group_b(g, carry):
            b = g // HKV
            hk = g % HKV

            @pl.when(jnp.logical_and(g >= WA0, g < WA0 + WAN))
            def _():
                per = 32 // WAN
                for r in range(per):
                    i = (g - WA0) * per + r
                    start_wq_piece(wqa_hbm, wqa_buf, i, w_sem.at[2])
                    start_wo_piece(woa_hbm, woa_buf, i, w_sem.at[3])

            q = None
            for r in range(REP):
                qr = jnp.broadcast_to(q_tab[hk * REP + r, pl.ds(b, 1), :], (8, DH))
                q = qr if r == 0 else jnp.where(row_h == r, qr, q)
            q = q.astype(bf16)

            def nxt(j, kslot, vslot):
                ck = g * NCH + j + NS

                @pl.when(ck < NCB)
                def _():
                    start_pair(kb_hbm, ck, kslot, vb_hbm, ck - 1, vslot)

                @pl.when(ck == NCB)
                def _():
                    start_pair(ka_hbm, 0, kslot, vb_hbm, NCB - 1, vslot)

                @pl.when(ck > NCB)
                def _():
                    start_pair(ka_hbm, ck - NCB, kslot, va_hbm, ck - NCB - 1, vslot)

            o = attend(q, g * NCH, nxt)
            o = o.astype(bf16).astype(f32)

            @pl.when(g == 0)
            def _():
                wait_all(wob_buf, w_sem.at[1])

            lhs = jnp.concatenate([jnp.broadcast_to(o[r:r + 1, :], (8, DH)) for r in range(REP)], axis=1)
            w = wob_buf[pl.ds(pl.multiple_of(hk * REP * DH, REP * DH), REP * DH), :]
            res = jnp.dot(lhs.astype(bf16), w, preferred_element_type=f32)
            acc_ref[...] += jnp.where(row_d == b, res * gb_tab[...], 0.0)
            return carry

        wait_all(wqb_buf, w_sem.at[0])
        fill_q_tab(wqb_buf)
        lax.fori_loop(0, NGB, group_b, 0)

        wait_all(wqa_buf, w_sem.at[2])
        fill_q_tab(wqa_buf)
        wait_all(woa_buf, w_sem.at[3])

        def group_a(g, carry):
            b = g // H
            h = g % H
            q = jnp.broadcast_to(q_tab[h, pl.ds(b, 1), :], (8, DH)).astype(bf16)

            def nxt(j, kslot, vslot):
                ck = g * NCH + j + NS

                @pl.when(ck < NCA)
                def _():
                    start_pair(ka_hbm, ck, kslot, va_hbm, ck - 1, vslot)

                @pl.when(ck == NCA)
                def _():
                    start_alone(va_hbm, NCA - 1, vbuf, 1, vslot)

            o = attend(q, NCB + g * NCH, nxt).astype(bf16)
            w = woa_buf[pl.ds(pl.multiple_of(h * DH, DH), DH), :]
            res = jnp.dot(o, w, preferred_element_type=f32)
            acc_ref[...] += jnp.where(row_d == b, res * ga_tab[...], 0.0)
            return carry

        lax.fori_loop(0, NGA, group_a, 0)

        out_ref[...] = acc_ref[0:NB, :].astype(out_ref.dtype)

    scratch = [
        pltpu.VMEM((NS, CH, DH), bf16),
        pltpu.VMEM((NS, CH, DH), bf16),
        pltpu.VMEM((D, H * DH), bf16),
        pltpu.VMEM((D, H * DH), bf16),
        pltpu.VMEM((H * DH, D), bf16),
        pltpu.VMEM((H * DH, D), bf16),
        pltpu.VMEM((NB, D), bf16),
        pltpu.VMEM((D,), bf16),
        pltpu.VMEM((H, 8, DH), f32),
        pltpu.VMEM((8, D), f32),
        pltpu.VMEM((8, D), f32),
        pltpu.VMEM((8, D), f32),
        pltpu.SemaphoreType.DMA((2, NS)),
        pltpu.SemaphoreType.DMA((4,)),
        pltpu.SemaphoreType.DMA((2,)),
    ]

    def run(A_x, A_k_cache, A_v_cache, A_wq, A_wo, B_x, B_k_cache, B_v_cache, B_wq, B_wo, gate_w):
        ka = A_k_cache.reshape(NGA * S, DH)
        va = A_v_cache.reshape(NGA * S, DH)
        kb = B_k_cache.reshape(NGB * S, DH)
        vb = B_v_cache.reshape(NGB * S, DH)
        any_spec = pl.BlockSpec(memory_space=pl.ANY)
        return pl.pallas_call(
            kernel,
            out_shape=jax.ShapeDtypeStruct((NB, D), bf16),
            in_specs=[any_spec] * 10,
            out_specs=pl.BlockSpec(memory_space=pltpu.VMEM),
            scratch_shapes=scratch,
            compiler_params=pltpu.CompilerParams(vmem_limit_bytes=100 * 1024 * 1024, disable_bounds_checks=True),
        )(A_x.reshape(NB, D), ka, va, A_wq, A_wo, kb, vb, B_wq, B_wo, gate_w).reshape(NB, 1, D)
    return run


_run = _make_kernel(NS=6)


@jax.jit
def pallas_gated_mix__mha_block_cached__gqa_block_cached__decode_kernel(
    A_x, A_k_cache, A_v_cache, A_wq, A_wo, B_x, B_k_cache, B_v_cache, B_wq, B_wo, gate_w,
):
    return _run(A_x, A_k_cache, A_v_cache, A_wq, A_wo, B_x, B_k_cache, B_v_cache, B_wq, B_wo, gate_w)
```

```python
import functools
import jax
import jax.numpy as jnp
from jax import lax
from jax.experimental import pallas as pl
from jax.experimental.pallas import tpu as pltpu

NB = 4
D = 512
H = 32
HKV = 8
S = 8192
DH = 128
NGA = NB * H
NGB = NB * HKV
REP = H // HKV


def split(start, n, R):
    out = []
    while n > 0:
        r = min(R, n)
        out.append((start, r)); start += r; n -= r
    return out


def _make_kernel(CH=2048, NS=6, R=128, NSTR=4, rot=0, dbg=None, WA0=8, WAN=16, swap=False, semchk=False):
    NCH = S // CH
    NCA = NGA * NCH
    NCB = NGB * NCH
    scale = DH ** -0.5
    f32 = jnp.float32
    bf16 = jnp.bfloat16

    G = CH // NSTR
    SEP = S // NSTR
    ks = [(i * SEP + r0, i * G + r0, n) for (r0, n) in split(0, G, R) for i in range(NSTR)]
    vs = ks[rot:] + ks[:rot]
    TK, TV = (1, 0) if swap else (0, 1)

    def kernel(xa_hbm, ka_hbm, va_hbm, wqa_hbm, woa_hbm, kb_hbm, vb_hbm, wqb_hbm, wob_hbm, gw_hbm,
               out_ref,
               kbuf, vbuf, wqa_buf, wqb_buf, woa_buf, wob_buf, xa_buf, gw_buf,
               q_tab, ga_tab, gb_tab, acc_ref,
               kv_sem, w_sem, s_sem):

        def slot_of(cg):
            return cg % NS if isinstance(cg, int) else lax.rem(cg, NS)

        def chunk_base(c):
            return (c // NCH) * S + (c % NCH) * G

        def kv_copy(src, base, buf, which, slot, d):
            hoff, voff, n = d
            row = base + hoff
            if not isinstance(row, int):
                row = pl.multiple_of(row, 16)
            return pltpu.make_async_copy(src.at[pl.ds(row, n), :],
                                         buf.at[slot, pl.ds(voff, n), :], kv_sem.at[which, slot])

        def start_pair(k_src, kc, kslot, v_src, vc, vslot):
            if dbg == 'nodma':
                return
            kb_, vb_ = chunk_base(kc), chunk_base(vc)
            for dk, dv in zip(ks, vs):
                kv_copy(k_src, kb_, kbuf, 0, kslot, dk).start(priority=TK)
                kv_copy(v_src, vb_, vbuf, 1, vslot, dv).start(priority=TV)

        def start_alone(src, c, buf, which, slot):
            if dbg == 'nodma':
                return
            base = chunk_base(c)
            for i, d in enumerate(ks):
                kv_copy(src, base, buf, which, slot, d).start(priority=i % 2)

        def wait_k(slot):
            if dbg == 'nodma':
                return
            pltpu.make_async_copy(kbuf.at[slot], kbuf.at[slot], kv_sem.at[0, slot]).wait()

        def wait_v(slot):
            if dbg == 'nodma':
                return
            pltpu.make_async_copy(vbuf.at[slot], vbuf.at[slot], kv_sem.at[1, slot]).wait()

        def start_wq_piece(src, buf, rblk, sem):
            row = rblk * 16
            if not isinstance(row, int):
                row = pl.multiple_of(row, 16)
            for c in range(4):
                pltpu.make_async_copy(src.at[pl.ds(row, 16), pl.ds(c * 1024, 1024)],
                                      buf.at[pl.ds(row, 16), pl.ds(c * 1024, 1024)], sem).start(priority=c % 2)

        def start_wo_piece(src, buf, rblk, sem):
            for r in range(4):
                row = rblk * 128 + r * 32
                if not isinstance(row, int):
                    row = pl.multiple_of(row, 32)
                pltpu.make_async_copy(src.at[pl.ds(row, 32), :],
                                      buf.at[pl.ds(row, 32), :], sem).start(priority=r % 2)

        def wait_all(buf, sem):
            pltpu.make_async_copy(buf, buf, sem).wait()

        cxa = pltpu.make_async_copy(xa_hbm, xa_buf, s_sem.at[0])
        cgw = pltpu.make_async_copy(gw_hbm, gw_buf, s_sem.at[1])
        cxa.start(); cgw.start()
        for i in range(32):
            start_wq_piece(wqb_hbm, wqb_buf, i, w_sem.at[0])
        start_alone(kb_hbm, 0, kbuf, 0, 0)
        for c in range(1, NS):
            start_pair(kb_hbm, c, c, vb_hbm, c - 1, c - 1)
        for i in range(32):
            start_wo_piece(wob_hbm, wob_buf, i, w_sem.at[1])

        cxa.wait(); cgw.wait()
        xa = xa_buf[...].astype(f32)
        gw = gw_buf[...].astype(f32).reshape(1, D)
        gate = jax.nn.sigmoid(jnp.sum(xa * gw, axis=1, keepdims=True))
        x8 = jnp.concatenate([xa, jnp.zeros((8 - NB, D), f32)], axis=0).astype(bf16)

        def fill_q_tab(wq_buf):
            q_all = jnp.dot(x8, wq_buf[...], preferred_element_type=f32)
            for h in range(H):
                q_tab[h] = q_all[:, h * DH:(h + 1) * DH]

        gate8 = jnp.concatenate([gate, jnp.zeros((8 - NB, 1), f32)], axis=0)
        ga_tab[...] = jnp.broadcast_to(gate8, (8, D))
        gb_tab[...] = jnp.broadcast_to(1.0 - gate8, (8, D))
        acc_ref[...] = jnp.zeros_like(acc_ref)

        row_d = lax.broadcasted_iota(jnp.int32, (8, D), 0)
        row_h = lax.broadcasted_iota(jnp.int32, (8, DH), 0) % REP

        def attend(q, cg0, next_src):
            m = l = acc = None
            for j in range(NCH):
                slot = slot_of(cg0 + j)
                wait_k(slot)
                s = lax.dot_general(q, kbuf[slot], (((1,), (1,)), ((), ())), preferred_element_type=f32) * scale
                next_src(j, slot, slot_of(cg0 + j + NS - 1))
                m_c = jnp.max(s, axis=1, keepdims=True)
                m_new = m_c if j == 0 else jnp.maximum(m, m_c)
                p = jnp.exp(s - m_new)
                l_c = jnp.sum(p, axis=1, keepdims=True)
                wait_v(slot)
                pv_ = jnp.dot(p.astype(bf16), vbuf[slot], preferred_element_type=f32)
                if j == 0:
                    l, acc = l_c, pv_
                else:
                    alpha = jnp.exp(m - m_new)
                    l = alpha * l + l_c
                    acc = alpha * acc + pv_
                m = m_new
            return (acc / l)

        def group_b(g, carry):
            b = g // HKV
            hk = g % HKV

            @pl.when(jnp.logical_and(g >= WA0, g < WA0 + WAN))
            def _():
                per = 32 // WAN
                for r in range(per):
                    i = (g - WA0) * per + r
                    start_wq_piece(wqa_hbm, wqa_buf, i, w_sem.at[2])
                    start_wo_piece(woa_hbm, woa_buf, i, w_sem.at[3])

            q = None
            for r in range(REP):
                qr = jnp.broadcast_to(q_tab[hk * REP + r, pl.ds(b, 1), :], (8, DH))
                q = qr if r == 0 else jnp.where(row_h == r, qr, q)
            q = q.astype(bf16)

            def nxt(j, kslot, vslot):
                ck = g * NCH + j + NS

                @pl.when(ck < NCB)
                def _():
                    start_pair(kb_hbm, ck, kslot, vb_hbm, ck - 1, vslot)

                @pl.when(ck == NCB)
                def _():
                    start_pair(ka_hbm, 0, kslot, vb_hbm, NCB - 1, vslot)

                @pl.when(ck > NCB)
                def _():
                    start_pair(ka_hbm, ck - NCB, kslot, va_hbm, ck - NCB - 1, vslot)

            o = attend(q, g * NCH, nxt)
            o = o.astype(bf16).astype(f32)

            @pl.when(g == 0)
            def _():
                wait_all(wob_buf, w_sem.at[1])

            lhs = jnp.concatenate([jnp.broadcast_to(o[r:r + 1, :], (8, DH)) for r in range(REP)], axis=1)
            w = wob_buf[pl.ds(pl.multiple_of(hk * REP * DH, REP * DH), REP * DH), :]
            res = jnp.dot(lhs.astype(bf16), w, preferred_element_type=f32)
            acc_ref[...] += jnp.where(row_d == b, res * gb_tab[...], 0.0)
            return carry

        wait_all(wqb_buf, w_sem.at[0])
        fill_q_tab(wqb_buf)
        lax.fori_loop(0, NGB, group_b, 0)

        wait_all(wqa_buf, w_sem.at[2])
        fill_q_tab(wqa_buf)
        wait_all(woa_buf, w_sem.at[3])

        def group_a(g, carry):
            b = g // H
            h = g % H
            q = jnp.broadcast_to(q_tab[h, pl.ds(b, 1), :], (8, DH)).astype(bf16)

            def nxt(j, kslot, vslot):
                ck = g * NCH + j + NS

                @pl.when(ck < NCA)
                def _():
                    start_pair(ka_hbm, ck, kslot, va_hbm, ck - 1, vslot)

                @pl.when(ck == NCA)
                def _():
                    start_alone(va_hbm, NCA - 1, vbuf, 1, vslot)

            o = attend(q, NCB + g * NCH, nxt).astype(bf16)
            w = woa_buf[pl.ds(pl.multiple_of(h * DH, DH), DH), :]
            res = jnp.dot(o, w, preferred_element_type=f32)
            acc_ref[...] += jnp.where(row_d == b, res * ga_tab[...], 0.0)
            return carry

        lax.fori_loop(0, NGA, group_a, 0)

        out_ref[...] = acc_ref[0:NB, :].astype(out_ref.dtype)

    scratch = [
        pltpu.VMEM((NS, CH, DH), bf16),
        pltpu.VMEM((NS, CH, DH), bf16),
        pltpu.VMEM((D, H * DH), bf16),
        pltpu.VMEM((D, H * DH), bf16),
        pltpu.VMEM((H * DH, D), bf16),
        pltpu.VMEM((H * DH, D), bf16),
        pltpu.VMEM((NB, D), bf16),
        pltpu.VMEM((D,), bf16),
        pltpu.VMEM((H, 8, DH), f32),
        pltpu.VMEM((8, D), f32),
        pltpu.VMEM((8, D), f32),
        pltpu.VMEM((8, D), f32),
        pltpu.SemaphoreType.DMA((2, NS)),
        pltpu.SemaphoreType.DMA((4,)),
        pltpu.SemaphoreType.DMA((2,)),
    ]

    def run(A_x, A_k_cache, A_v_cache, A_wq, A_wo, B_x, B_k_cache, B_v_cache, B_wq, B_wo, gate_w):
        ka = A_k_cache.reshape(NGA * S, DH)
        va = A_v_cache.reshape(NGA * S, DH)
        kb = B_k_cache.reshape(NGB * S, DH)
        vb = B_v_cache.reshape(NGB * S, DH)
        any_spec = pl.BlockSpec(memory_space=pl.ANY)
        return pl.pallas_call(
            kernel,
            out_shape=jax.ShapeDtypeStruct((NB, D), bf16),
            in_specs=[any_spec] * 10,
            out_specs=pl.BlockSpec(memory_space=pltpu.VMEM),
            scratch_shapes=scratch,
            compiler_params=pltpu.CompilerParams(vmem_limit_bytes=100 * 1024 * 1024, disable_bounds_checks=True, disable_semaphore_checks=not semchk),
        )(A_x.reshape(NB, D), ka, va, A_wq, A_wo, kb, vb, B_wq, B_wo, gate_w).reshape(NB, 1, D)
    return run


_run = _make_kernel(NS=6)


@jax.jit
def pallas_gated_mix__mha_block_cached__gqa_block_cached__decode_kernel(
    A_x, A_k_cache, A_v_cache, A_wq, A_wo, B_x, B_k_cache, B_v_cache, B_wq, B_wo, gate_w,
):
    return _run(A_x, A_k_cache, A_v_cache, A_wq, A_wo, B_x, B_k_cache, B_v_cache, B_wq, B_wo, gate_w)
```

```python
import functools
import jax
import jax.numpy as jnp
from jax import lax
from jax.experimental import pallas as pl
from jax.experimental.pallas import tpu as pltpu

NB = 4
D = 512
H = 32
HKV = 8
S = 8192
DH = 128
REP = H // HKV
NSTR = 4
NUA = NB * H // NSTR
NUB = NB * HKV // NSTR
R = 128


def _make_kernel(G=512, LB=4, LA=5, dbg=None, WPS=2, unroll=1, semchk=False, pts=4, NPRE=3):
    NS = max(LB, LA) + 1
    SPU = S // G
    NTA = NUA * SPU
    NTB = NUB * SPU
    CH = NSTR * G
    NP = G // R
    scale = DH ** -0.5
    f32 = jnp.float32
    bf16 = jnp.bfloat16
    NEG = -1e30
    NFILL = 4
    assert LA == LB or LA == LB + 1

    rr = [(i, a) for a in range(NP) for i in range(NSTR)]
    seq = [(i, a) for i in range(NSTR) for a in range(NP)]

    def kernel(xa_hbm, ka_hbm, va_hbm, wqa_hbm, woa_hbm, kb_hbm, vb_hbm, wqb_hbm, wob_hbm, gw_hbm,
               out_ref,
               kbuf, vbuf, wqa_buf, wqb_buf, woa_buf, wob_buf, xa_buf, gw_buf,
               q_tab, ga_tab, gb_tab, acc_ref,
               k_sem, v_sem, w_sem, s_sem):

        def slot_of(t):
            return t % NS if isinstance(t, int) else lax.rem(t, NS)

        def step_base(t):
            return (t // SPU) * (NSTR * S) + (t % SPU) * G

        def kv_copy(src, base, buf, sem, slot, i, a):
            row = base + (i * S + a * R)
            if not isinstance(row, int):
                row = pl.multiple_of(row, R)
            return pltpu.make_async_copy(src.at[pl.ds(row, R), :],
                                         buf.at[slot, pl.ds(i * G + a * R, R), :], sem)

        def part_of(lst, part, nparts):
            if part is None:
                return list(enumerate(lst))
            n = len(lst) // nparts
            return list(enumerate(lst))[part * n:(part + 1) * n]

        def start_pair(k_src, kt, v_src, vt, gstep, part=None, nparts=1):
            if dbg == 'nodma':
                return
            kslot, vslot = slot_of(gstep), slot_of(gstep - 1)
            kb_, vb_ = step_base(kt), step_base(vt)
            for _, (i, a) in part_of(rr, part, nparts):
                kv_copy(k_src, kb_, kbuf, k_sem.at[kslot], kslot, i, a).start(priority=0)
                kv_copy(v_src, vb_, vbuf, v_sem.at[vslot, i], vslot, i, a).start(priority=1)

        def start_k_alone(src, t, slot):
            if dbg == 'nodma':
                return
            base = step_base(t)
            for n, (i, a) in enumerate(rr):
                kv_copy(src, base, kbuf, k_sem.at[slot], slot, i, a).start(priority=n % 2)

        def start_v_alone(src, t, slot, part=None, nparts=1):
            if dbg == 'nodma':
                return
            base = step_base(t)
            for n, (i, a) in part_of(seq, part, nparts):
                kv_copy(src, base, vbuf, v_sem.at[slot, i], slot, i, a).start(priority=n % 2)

        def wait_k(slot):
            if dbg == 'nodma':
                return
            pltpu.make_async_copy(kbuf.at[slot], kbuf.at[slot], k_sem.at[slot]).wait()

        def wait_v(slot, i):
            if dbg == 'nodma':
                return
            v = vbuf.at[slot, pl.ds(i * G, G), :]
            pltpu.make_async_copy(v, v, v_sem.at[slot, i]).wait()

        def start_w_pair(wq_src, wq_dst, wq_sem, wo_src, wo_dst, wo_sem, n):
            p = (n % 4) * 32 + n // 4
            r = (p // 4) * 16
            c = (p % 4) * 1024
            ro = p * 32
            if not isinstance(n, int):
                r = pl.multiple_of(r, 16)
                c = pl.multiple_of(c, 1024)
                ro = pl.multiple_of(ro, 32)
            pltpu.make_async_copy(wq_src.at[pl.ds(r, 16), pl.ds(c, 1024)],
                                  wq_dst.at[pl.ds(r, 16), pl.ds(c, 1024)], wq_sem).start(priority=0)
            pltpu.make_async_copy(wo_src.at[pl.ds(ro, 32), :],
                                  wo_dst.at[pl.ds(ro, 32), :], wo_sem).start(priority=1)

        def wait_all(buf, sem):
            pltpu.make_async_copy(buf, buf, sem).wait()

        cxa = pltpu.make_async_copy(xa_hbm, xa_buf, s_sem.at[0])
        cgw = pltpu.make_async_copy(gw_hbm, gw_buf, s_sem.at[1])
        cxa.start(priority=0); cgw.start(priority=1)
        for n in range(128):
            start_w_pair(wqb_hbm, wqb_buf, w_sem.at[0], wob_hbm, wob_buf, w_sem.at[1], n)
        start_k_alone(kb_hbm, 0, 0)
        for t in range(1, LB - 1):
            start_pair(kb_hbm, t, vb_hbm, t - 1, t)

        cxa.wait(); cgw.wait()
        xa = xa_buf[...].astype(f32)
        gw = gw_buf[...].astype(f32).reshape(1, D)
        gate = jax.nn.sigmoid(jnp.sum(xa * gw, axis=1, keepdims=True))
        x8 = jnp.concatenate([xa, jnp.zeros((8 - NB, D), f32)], axis=0).astype(bf16)
        gate8 = jnp.concatenate([gate, jnp.zeros((8 - NB, 1), f32)], axis=0)
        ga_tab[...] = jnp.broadcast_to(gate8, (8, D))
        gb_tab[...] = jnp.broadcast_to(1.0 - gate8, (8, D))
        acc_ref[...] = jnp.zeros_like(acc_ref)

        row_d = lax.broadcasted_iota(jnp.int32, (8, D), 0)
        row_g = lax.broadcasted_iota(jnp.int32, (8, G), 0)
        row_h = lax.broadcasted_iota(jnp.int32, (8, DH), 0)

        def fill_q_tab(wq_buf, dup, issue):
            per = 4 if dup else 8
            hp = H // NFILL
            for k in range(NFILL):
                issue(k)
                q_p = jnp.dot(x8, wq_buf[:, k * hp * DH:(k + 1) * hp * DH], preferred_element_type=f32)
                for b in range(NB):
                    for j in range(hp // per):
                        rows = [q_p[b:b + 1, (j * per + r) * DH:(j * per + r + 1) * DH] for r in range(per)]
                        if dup:
                            rows = rows + rows
                        q_tab[b * (H // per) + k * (hp // per) + j] = jnp.concatenate(rows, axis=0)

        def pick(vals, rows, div):
            out = vals[-1]
            for k in range(len(vals) - 2, -1, -1):
                out = jnp.where(div(rows) == k, vals[k], out)
            return out

        def step(t, qs, streams, state, next_src):
            slot = slot_of(t)
            issued = [0]

            def issue():
                next_src(issued[0])
                issued[0] += 1

            wait_k(slot)
            sv = {}
            for j, (q, st) in enumerate(zip(qs, streams)):
                for i in st:
                    sv[i] = lax.dot_general(q, kbuf[slot, pl.ds(i * G, G), :], (((1,), (1,)), ((), ())),
                                            preferred_element_type=f32)
                    if pts == 8 or (pts == 4 and i % 2 == 1) or (pts in (1, 2) and i == 3):
                        issue()
            ss = []
            for j, st in enumerate(streams):
                vals = [sv[i] for i in st]
                if len(st) == 4:
                    ss.append(pick(vals, row_g, lambda r: r % 4))
                else:
                    ss.append(pick(vals, row_g, lambda r: r // 4))
            ps, mid = [], []
            for s, (m, l, acc) in zip(ss, state):
                m_new = jnp.maximum(m, jnp.max(s, axis=1, keepdims=True))
                p = jnp.exp((s - m_new) * scale)
                alpha = jnp.exp((m - m_new) * scale)
                lp = p[:, 0:DH]
                for k in range(1, G // DH):
                    lp = lp + p[:, k * DH:(k + 1) * DH]
                ps.append(p.astype(bf16))
                mid.append((m_new, alpha * l + lp, alpha * acc))
            pvs = {}
            for j, st in enumerate(streams):
                for i in st:
                    wait_v(slot, i)
                    pvs[i] = jnp.dot(ps[j], vbuf[slot, pl.ds(i * G, G), :], preferred_element_type=f32)
                    if pts == 8 or (pts == 4 and i % 2 == 1) or (pts == 2 and i == 3):
                        issue()
            assert issued[0] == pts
            new = []
            for j, st in enumerate(streams):
                vals = [pvs[i] for i in st]
                if len(st) == 4:
                    pv = pick(vals, row_h, lambda r: r % 4)
                else:
                    pv = pick(vals, row_h, lambda r: r // 4)
                m_new, l, acc = mid[j]
                new.append((m_new, l, acc + pv))
            return new

        def init_state(n):
            return [(jnp.full((8, 1), NEG, f32), jnp.zeros((8, DH), f32), jnp.zeros((8, DH), f32)) for _ in range(n)]

        def finish(st):
            m, l, acc = st
            return (acc / jnp.sum(l, axis=1, keepdims=True)).astype(bf16).astype(f32)

        def project(o, nrows, w):
            lhs = jnp.concatenate([jnp.broadcast_to(o[r:r + 1, :], (8, DH)) for r in range(nrows)], axis=1)
            return jnp.dot(lhs.astype(bf16), w, preferred_element_type=f32)

        def flat(state):
            return tuple(x for st in state for x in st)

        def unflat(vals):
            return [tuple(vals[3 * j:3 * j + 3]) for j in range(len(vals) // 3)]

        def unit_b(u, carry, cond=True):
            b = u // 2
            half = u % 2
            qs = [q_tab[b * 4 + half * 2 + j].astype(bf16) for j in range(2)]

            def body(c, vals):
                t = u * SPU + c

                @pl.when(t < 128 // WPS)
                def _():
                    for r in range(WPS):
                        start_w_pair(wqa_hbm, wqa_buf, w_sem.at[2], woa_hbm, woa_buf, w_sem.at[3], t * WPS + r)

                def nxt(part):
                    ck = t + LB
                    if not cond:
                        start_pair(kb_hbm, ck, vb_hbm, ck - 1, ck, part, pts)
                        return

                    @pl.when(ck < NTB)
                    def _():
                        start_pair(kb_hbm, ck, vb_hbm, ck - 1, ck, part, pts)

                    @pl.when(ck == NTB)
                    def _():
                        start_pair(ka_hbm, 0, vb_hbm, NTB - 1, ck, part, pts)

                    @pl.when(ck > NTB)
                    def _():
                        start_pair(ka_hbm, ck - NTB, va_hbm, ck - NTB - 1, ck, part, pts)

                return flat(step(t, qs, [[0, 1], [2, 3]], unflat(vals), nxt))

            vals = lax.fori_loop(0, SPU, body, flat(init_state(2)), unroll=unroll)
            st = unflat(vals)
            res = None
            for j in range(2):
                row0 = pl.multiple_of((half * 16 + j * 8) * DH, 8 * DH)
                r = project(finish(st[j]), 8, wob_buf[pl.ds(row0, 8 * DH), :])
                res = r if res is None else res + r
            acc_ref[...] += jnp.where(row_d == b, res * gb_tab[...], 0.0)
            return carry

        wait_all(wqb_buf, w_sem.at[0])
        fill_q_tab(wqb_buf, False,
                   lambda k: start_pair(kb_hbm, LB - 1, vb_hbm, LB - 2, LB - 1, k, NFILL))
        wait_all(wob_buf, w_sem.at[1])
        lax.fori_loop(0, NUB - 1, functools.partial(unit_b, cond=False), 0)
        unit_b(NUB - 1, 0)

        wait_all(wqa_buf, w_sem.at[2])
        if LA == LB + 1:
            fill_q_tab(wqa_buf, True,
                       lambda k: start_pair(ka_hbm, LB, va_hbm, LB - 1, NTB + LB, k, NFILL))
        else:
            fill_q_tab(wqa_buf, True, lambda k: None)
        wait_all(woa_buf, w_sem.at[3])

        def unit_a(u, carry, cond=True):
            b = u // 8
            hq = u % 8
            qs = [q_tab[u].astype(bf16)]

            def body(c, vals):
                ta = u * SPU + c

                def nxt(part):
                    ck = ta + LA
                    if not cond:
                        start_pair(ka_hbm, ck, va_hbm, ck - 1, NTB + ck, part, pts)
                        return

                    @pl.when(ck < NTA)
                    def _():
                        start_pair(ka_hbm, ck, va_hbm, ck - 1, NTB + ck, part, pts)

                    @pl.when(ck == NTA)
                    def _():
                        start_v_alone(va_hbm, NTA - 1, slot_of(NTB + ck - 1), part, pts)

                return flat(step(NTB + ta, qs, [[0, 1, 2, 3]], unflat(vals), nxt))

            vals = lax.fori_loop(0, SPU, body, flat(init_state(1)), unroll=unroll)
            row0 = pl.multiple_of(hq * 4 * DH, 4 * DH)
            res = project(finish(unflat(vals)[0]), 4, woa_buf[pl.ds(row0, 4 * DH), :])
            acc_ref[...] += jnp.where(row_d == b, res * ga_tab[...], 0.0)
            return carry

        lax.fori_loop(0, NUA - 1, functools.partial(unit_a, cond=False), 0)
        unit_a(NUA - 1, 0)

        out_ref[...] = acc_ref[0:NB, :].astype(out_ref.dtype)

    scratch = [
        pltpu.VMEM((NS, CH, DH), bf16),
        pltpu.VMEM((NS, CH, DH), bf16),
        pltpu.VMEM((D, H * DH), bf16),
        pltpu.VMEM((D, H * DH), bf16),
        pltpu.VMEM((H * DH, D), bf16),
        pltpu.VMEM((H * DH, D), bf16),
        pltpu.VMEM((NB, D), bf16),
        pltpu.VMEM((D,), bf16),
        pltpu.VMEM((NUA, 8, DH), f32),
        pltpu.VMEM((8, D), f32),
        pltpu.VMEM((8, D), f32),
        pltpu.VMEM((8, D), f32),
        pltpu.SemaphoreType.DMA((NS,)),
        pltpu.SemaphoreType.DMA((NS, NSTR)),
        pltpu.SemaphoreType.DMA((4,)),
        pltpu.SemaphoreType.DMA((2,)),
    ]

    def run(A_x, A_k_cache, A_v_cache, A_wq, A_wo, B_x, B_k_cache, B_v_cache, B_wq, B_wo, gate_w):
        ka = A_k_cache.reshape(NB * H * S, DH)
        va = A_v_cache.reshape(NB * H * S, DH)
        kb = B_k_cache.reshape(NB * HKV * S, DH)
        vb = B_v_cache.reshape(NB * HKV * S, DH)
        any_spec = pl.BlockSpec(memory_space=pl.ANY)
        return pl.pallas_call(
            kernel,
            out_shape=jax.ShapeDtypeStruct((NB, D), bf16),
            in_specs=[any_spec] * 10,
            out_specs=pl.BlockSpec(memory_space=pltpu.VMEM),
            scratch_shapes=scratch,
            compiler_params=pltpu.CompilerParams(vmem_limit_bytes=100 * 1024 * 1024, disable_bounds_checks=True,
                                                 disable_semaphore_checks=not semchk),
        )(A_x.reshape(NB, D), ka, va, A_wq, A_wo, kb, vb, B_wq, B_wo, gate_w).reshape(NB, 1, D)
    return run


_run = _make_kernel(pts=1)


@jax.jit
def pallas_gated_mix__mha_block_cached__gqa_block_cached__decode_kernel(
    A_x, A_k_cache, A_v_cache, A_wq, A_wo, B_x, B_k_cache, B_v_cache, B_wq, B_wo, gate_w,
):
    return _run(A_x, A_k_cache, A_v_cache, A_wq, A_wo, B_x, B_k_cache, B_v_cache, B_wq, B_wo, gate_w)
```

```python
import functools
import jax
import jax.numpy as jnp
from jax import lax
from jax.experimental import pallas as pl
from jax.experimental.pallas import tpu as pltpu

NB = 4
D = 512
H = 32
HKV = 8
S = 8192
DH = 128
REP = H // HKV
NSTR = 4
NUA = NB * H // NSTR
NUB = NB * HKV // NSTR
R = 128


def _make_kernel(G=512, LB=4, LA=5, dbg=None, WPS=2, unroll=1, semchk=False, pts=1, NPRE=3, tail2=True, dbl=True):
    NS = max(LB, LA) + 1
    SPU = S // G
    NTA = NUA * SPU
    NTB = NUB * SPU
    CH = NSTR * G
    NP = G // R
    scale = DH ** -0.5
    f32 = jnp.float32
    bf16 = jnp.bfloat16
    NEG = -1e30
    NFILL = 4
    assert LA == LB or LA == LB + 1

    rr = [(i, a) for a in range(NP) for i in range(NSTR)]
    seq = [(i, a) for i in range(NSTR) for a in range(NP)]

    def kernel(xa_hbm, ka_hbm, va_hbm, wqa_hbm, woa_hbm, kb_hbm, vb_hbm, wqb_hbm, wob_hbm, gw_hbm,
               out_ref,
               kbuf, vbuf, wqa_buf, wqb_buf, woa_buf, wob_buf, xa_buf, gw_buf,
               q_tab, ga_tab, gb_tab, acc_ref,
               k_sem, v_sem, w_sem, s_sem):

        def slot_of(t):
            return t % NS if isinstance(t, int) else lax.rem(t, NS)

        def step_base(t):
            return (t // SPU) * (NSTR * S) + (t % SPU) * G

        def kv_copy(src, base, buf, sem, slot, i, a):
            row = base + (i * S + a * R)
            if not isinstance(row, int):
                row = pl.multiple_of(row, R)
            return pltpu.make_async_copy(src.at[pl.ds(row, R), :],
                                         buf.at[slot, pl.ds(i * G + a * R, R), :], sem)

        def part_of(lst, part, nparts):
            if part is None:
                return list(enumerate(lst))
            n = len(lst) // nparts
            return list(enumerate(lst))[part * n:(part + 1) * n]

        def start_pair(k_src, kt, v_src, vt, gstep, part=None, nparts=1):
            if dbg == 'nodma':
                return
            kslot, vslot = slot_of(gstep), slot_of(gstep - 1)
            kb_, vb_ = step_base(kt), step_base(vt)
            for _, (i, a) in part_of(rr, part, nparts):
                kv_copy(k_src, kb_, kbuf, k_sem.at[kslot], kslot, i, a).start(priority=0)
                kv_copy(v_src, vb_, vbuf, v_sem.at[vslot], vslot, i, a).start(priority=1)

        def start_k_alone(src, t, slot, part=None, nparts=1):
            if dbg == 'nodma':
                return
            base = step_base(t)
            for n, (i, a) in part_of(rr, part, nparts):
                kv_copy(src, base, kbuf, k_sem.at[slot], slot, i, a).start(priority=n % 2)

        def start_v_alone(src, t, slot, part=None, nparts=1):
            if dbg == 'nodma':
                return
            base = step_base(t)
            for n, (i, a) in part_of(rr, part, nparts):
                kv_copy(src, base, vbuf, v_sem.at[slot], slot, i, a).start(priority=n % 2)

        def wait_k(slot):
            if dbg == 'nodma':
                return
            pltpu.make_async_copy(kbuf.at[slot], kbuf.at[slot], k_sem.at[slot]).wait()

        def wait_v(slot):
            if dbg == 'nodma':
                return
            pltpu.make_async_copy(vbuf.at[slot], vbuf.at[slot], v_sem.at[slot]).wait()

        def start_w_pair(wq_src, wq_dst, wq_sem, wo_src, wo_dst, wo_sem, n):
            p = (n % 4) * 32 + n // 4
            r = (p // 4) * 16
            c = (p % 4) * 1024
            ro = p * 32
            if not isinstance(n, int):
                r = pl.multiple_of(r, 16)
                c = pl.multiple_of(c, 1024)
                ro = pl.multiple_of(ro, 32)
            pltpu.make_async_copy(wq_src.at[pl.ds(r, 16), pl.ds(c, 1024)],
                                  wq_dst.at[pl.ds(r, 16), pl.ds(c, 1024)], wq_sem).start(priority=0)
            pltpu.make_async_copy(wo_src.at[pl.ds(ro, 32), :],
                                  wo_dst.at[pl.ds(ro, 32), :], wo_sem).start(priority=1)

        def wait_all(buf, sem):
            pltpu.make_async_copy(buf, buf, sem).wait()

        cxa = pltpu.make_async_copy(xa_hbm, xa_buf, s_sem.at[0])
        cgw = pltpu.make_async_copy(gw_hbm, gw_buf, s_sem.at[1])
        cxa.start(priority=0); cgw.start(priority=1)
        for n in range(128):
            start_w_pair(wqb_hbm, wqb_buf, w_sem.at[0], wob_hbm, wob_buf, w_sem.at[1], n)
        start_k_alone(kb_hbm, 0, 0)
        for t in range(1, LB - 1):
            start_pair(kb_hbm, t, vb_hbm, t - 1, t)

        cxa.wait(); cgw.wait()
        xa = xa_buf[...].astype(f32)
        gw = gw_buf[...].astype(f32).reshape(1, D)
        gate = jax.nn.sigmoid(jnp.sum(xa * gw, axis=1, keepdims=True))
        x8 = jnp.concatenate([xa, jnp.zeros((8 - NB, D), f32)], axis=0).astype(bf16)
        gate8 = jnp.concatenate([gate, jnp.zeros((8 - NB, 1), f32)], axis=0)
        ga_tab[...] = jnp.broadcast_to(gate8, (8, D))
        gb_tab[...] = jnp.broadcast_to(1.0 - gate8, (8, D))
        acc_ref[...] = jnp.zeros_like(acc_ref)

        row_d = lax.broadcasted_iota(jnp.int32, (8, D), 0)
        row_g = lax.broadcasted_iota(jnp.int32, (8, G), 0)
        row_h = lax.broadcasted_iota(jnp.int32, (8, DH), 0)

        def fill_q_tab(wq_buf, dup, issue):
            per = 4 if dup else 8
            hp = H // NFILL
            for k in range(NFILL):
                issue(k)
                q_p = jnp.dot(x8, wq_buf[:, k * hp * DH:(k + 1) * hp * DH], preferred_element_type=f32)
                for b in range(NB):
                    for j in range(hp // per):
                        rows = [q_p[b:b + 1, (j * per + r) * DH:(j * per + r + 1) * DH] for r in range(per)]
                        if dup:
                            rows = rows + rows
                        q_tab[b * (H // per) + k * (hp // per) + j] = jnp.concatenate(rows, axis=0)

        def pick(vals, rows, div):
            out = vals[-1]
            for k in range(len(vals) - 2, -1, -1):
                out = jnp.where(div(rows) == k, vals[k], out)
            return out

        def step(ts, qs, streams, state, next_src):
            slots = [slot_of(t) for t in ts]
            issued = [0]

            def issue():
                next_src(issued[0])
                issued[0] += 1

            def sel(vals, rows, n):
                return pick(vals, rows, (lambda r: r % 4) if n == 4 else (lambda r: r // 4))

            ss = [[] for _ in qs]
            for slot in slots:
                wait_k(slot)
                for j, (q, st) in enumerate(zip(qs, streams)):
                    vals = [lax.dot_general(q, kbuf[slot, pl.ds(i * G, G), :], (((1,), (1,)), ((), ())),
                                            preferred_element_type=f32) for i in st]
                    ss[j].append(sel(vals, row_g, len(st)))
            issue()
            ps, mid = [], []
            for sl, (m, l, acc) in zip(ss, state):
                mx = sl[0]
                for s_ in sl[1:]:
                    mx = jnp.maximum(mx, s_)
                m_new = jnp.maximum(m, jnp.max(mx, axis=1, keepdims=True))
                alpha = jnp.exp((m - m_new) * scale)
                l = alpha * l
                pl_ = []
                for s_ in sl:
                    p = jnp.exp((s_ - m_new) * scale)
                    for k in range(G // DH):
                        l = l + p[:, k * DH:(k + 1) * DH]
                    pl_.append(p.astype(bf16))
                ps.append(pl_)
                mid.append((m_new, l, alpha * acc))
            accs = [x[2] for x in mid]
            for c, slot in enumerate(slots):
                wait_v(slot)
                for j, st in enumerate(streams):
                    vals = [jnp.dot(ps[j][c], vbuf[slot, pl.ds(i * G, G), :], preferred_element_type=f32)
                            for i in st]
                    accs[j] = accs[j] + sel(vals, row_h, len(st))
            if pts == 2:
                issue()
            assert issued[0] == pts
            return [(mid[j][0], mid[j][1], accs[j]) for j in range(len(qs))]

        def init_state(n):
            return [(jnp.full((8, 1), NEG, f32), jnp.zeros((8, DH), f32), jnp.zeros((8, DH), f32)) for _ in range(n)]

        def finish(st):
            m, l, acc = st
            return (acc / jnp.sum(l, axis=1, keepdims=True)).astype(bf16).astype(f32)

        def project(o, nrows, w):
            lhs = jnp.concatenate([jnp.broadcast_to(o[r:r + 1, :], (8, DH)) for r in range(nrows)], axis=1)
            return jnp.dot(lhs.astype(bf16), w, preferred_element_type=f32)

        def flat(state):
            return tuple(x for st in state for x in st)

        def unflat(vals):
            return [tuple(vals[3 * j:3 * j + 3]) for j in range(len(vals) // 3)]

        def unit_b(u, carry, cond=True):
            b = u // 2
            half = u % 2
            qs = [q_tab[b * 4 + half * 2 + j].astype(bf16) for j in range(2)]

            def body(c, vals):
                t = u * SPU + c

                @pl.when(t < 128 // WPS)
                def _():
                    for r in range(WPS):
                        start_w_pair(wqa_hbm, wqa_buf, w_sem.at[2], woa_hbm, woa_buf, w_sem.at[3], t * WPS + r)

                def nxt(part):
                    ck = t + LB
                    if not cond:
                        start_pair(kb_hbm, ck, vb_hbm, ck - 1, ck, part, pts)
                        return

                    @pl.when(ck < NTB)
                    def _():
                        start_pair(kb_hbm, ck, vb_hbm, ck - 1, ck, part, pts)

                    @pl.when(ck == NTB)
                    def _():
                        start_pair(ka_hbm, 0, vb_hbm, NTB - 1, ck, part, pts)

                    @pl.when(ck > NTB)
                    def _():
                        start_pair(ka_hbm, ck - NTB, va_hbm, ck - NTB - 1, ck, part, pts)

                return flat(step([t], qs, [[0, 1], [2, 3]], unflat(vals), nxt))

            vals = lax.fori_loop(0, SPU, body, flat(init_state(2)), unroll=unroll)
            st = unflat(vals)
            res = None
            for j in range(2):
                row0 = pl.multiple_of((half * 16 + j * 8) * DH, 8 * DH)
                r = project(finish(st[j]), 8, wob_buf[pl.ds(row0, 8 * DH), :])
                res = r if res is None else res + r
            acc_ref[...] += jnp.where(row_d == b, res * gb_tab[...], 0.0)
            return carry

        wait_all(wqb_buf, w_sem.at[0])
        fill_q_tab(wqb_buf, False,
                   lambda k: start_pair(kb_hbm, LB - 1, vb_hbm, LB - 2, LB - 1, k, NFILL))
        wait_all(wob_buf, w_sem.at[1])
        lax.fori_loop(0, NUB - 1, functools.partial(unit_b, cond=False), 0)
        unit_b(NUB - 1, 0)

        wait_all(wqa_buf, w_sem.at[2])
        if LA == LB + 1:
            fill_q_tab(wqa_buf, True,
                       lambda k: start_pair(ka_hbm, LB, va_hbm, LB - 1, NTB + LB, k, NFILL))
        else:
            fill_q_tab(wqa_buf, True, lambda k: None)
        wait_all(woa_buf, w_sem.at[3])

        def unit_a(u, carry, last=False):
            b = u // 8
            hq = u % 8
            qs = [q_tab[u].astype(bf16)]

            def body(c, vals, mode, n=1):
                ta = u * SPU + c

                def nxt(part):
                    ck = ta + LA
                    if mode == "pair":
                        start_pair(ka_hbm, ck, va_hbm, ck - 1, NTB + ck, part, pts)
                    elif mode == "valone":
                        start_v_alone(va_hbm, NTA - 1, slot_of(NTB + NTA - 1), part, pts)
                    elif mode == "kalone":
                        start_k_alone(ka_hbm, NTA - 1, slot_of(NTB + NTA - 1), part, pts)
                    elif mode == "vv":
                        if pts == 1:
                            start_v_alone(va_hbm, NTA - 2, slot_of(NTB + NTA - 2))
                            start_v_alone(va_hbm, NTA - 1, slot_of(NTB + NTA - 1))
                        else:
                            h = pts // 2
                            if part < h:
                                start_v_alone(va_hbm, NTA - 2, slot_of(NTB + NTA - 2), part, h)
                            else:
                                start_v_alone(va_hbm, NTA - 1, slot_of(NTB + NTA - 1), part - h, h)

                return flat(step([NTB + ta + k for k in range(n)], qs, [[0, 1, 2, 3]], unflat(vals), nxt))

            vals = flat(init_state(1))
            if not last:
                vals = lax.fori_loop(0, SPU, functools.partial(body, mode="pair"), vals, unroll=unroll)
            else:
                if tail2:
                    vals = lax.fori_loop(0, SPU - LA - 1, functools.partial(body, mode="pair"), vals)
                    vals = body(SPU - LA - 1, vals, "kalone")
                    vals = body(SPU - LA, vals, "vv")
                else:
                    vals = lax.fori_loop(0, SPU - LA, functools.partial(body, mode="pair"), vals)
                    vals = body(SPU - LA, vals, "valone")
                if dbl:
                    vals = lax.fori_loop(SPU - LA + 1, SPU - 2, functools.partial(body, mode="none"), vals)
                    vals = body(SPU - 2, vals, "none", n=2)
                else:
                    vals = lax.fori_loop(SPU - LA + 1, SPU, functools.partial(body, mode="none"), vals)
            row0 = pl.multiple_of(hq * 4 * DH, 4 * DH)
            res = project(finish(unflat(vals)[0]), 4, woa_buf[pl.ds(row0, 4 * DH), :])
            acc_ref[...] += jnp.where(row_d == b, res * ga_tab[...], 0.0)
            return carry

        lax.fori_loop(0, NUA - 1, unit_a, 0)
        unit_a(NUA - 1, 0, last=True)

        out_ref[...] = acc_ref[0:NB, :].astype(out_ref.dtype)

    scratch = [
        pltpu.VMEM((NS, CH, DH), bf16),
        pltpu.VMEM((NS, CH, DH), bf16),
        pltpu.VMEM((D, H * DH), bf16),
        pltpu.VMEM((D, H * DH), bf16),
        pltpu.VMEM((H * DH, D), bf16),
        pltpu.VMEM((H * DH, D), bf16),
        pltpu.VMEM((NB, D), bf16),
        pltpu.VMEM((D,), bf16),
        pltpu.VMEM((NUA, 8, DH), f32),
        pltpu.VMEM((8, D), f32),
        pltpu.VMEM((8, D), f32),
        pltpu.VMEM((8, D), f32),
        pltpu.SemaphoreType.DMA((NS,)),
        pltpu.SemaphoreType.DMA((NS,)),
        pltpu.SemaphoreType.DMA((4,)),
        pltpu.SemaphoreType.DMA((2,)),
    ]

    def run(A_x, A_k_cache, A_v_cache, A_wq, A_wo, B_x, B_k_cache, B_v_cache, B_wq, B_wo, gate_w):
        ka = A_k_cache.reshape(NB * H * S, DH)
        va = A_v_cache.reshape(NB * H * S, DH)
        kb = B_k_cache.reshape(NB * HKV * S, DH)
        vb = B_v_cache.reshape(NB * HKV * S, DH)
        any_spec = pl.BlockSpec(memory_space=pl.ANY)
        return pl.pallas_call(
            kernel,
            out_shape=jax.ShapeDtypeStruct((NB, D), bf16),
            in_specs=[any_spec] * 10,
            out_specs=pl.BlockSpec(memory_space=pltpu.VMEM),
            scratch_shapes=scratch,
            compiler_params=pltpu.CompilerParams(vmem_limit_bytes=100 * 1024 * 1024, disable_bounds_checks=True,
                                                 disable_semaphore_checks=not semchk),
        )(A_x.reshape(NB, D), ka, va, A_wq, A_wo, kb, vb, B_wq, B_wo, gate_w).reshape(NB, 1, D)
    return run


_run = _make_kernel()


@jax.jit
def pallas_gated_mix__mha_block_cached__gqa_block_cached__decode_kernel(
    A_x, A_k_cache, A_v_cache, A_wq, A_wo, B_x, B_k_cache, B_v_cache, B_wq, B_wo, gate_w,
):
    return _run(A_x, A_k_cache, A_v_cache, A_wq, A_wo, B_x, B_k_cache, B_v_cache, B_wq, B_wo, gate_w)
```

```python
import functools

import jax
import jax.numpy as jnp
from jax import lax
from jax.experimental import pallas as pl
from jax.experimental.pallas import tpu as pltpu

NB = 4
D = 512
H = 32
HKV = 8
S = 8192
DH = 128
NSTR = 4
NUA = NB * H // NSTR
NUB = NB * HKV // NSTR
R = 128
NW = 128


def _make_kernel(G=512, LB=4, WPS=2, semchk=False):
    LA = LB + 1
    NS = LA + 1
    SPU = S // G
    NTA = NUA * SPU
    NTB = NUB * SPU
    CH = NSTR * G
    NP = G // R
    NC = G // DH
    scale = DH ** -0.5
    f32 = jnp.float32
    bf16 = jnp.bfloat16
    NEG = -1e30
    NFILL = 4

    rr = [(i, a) for a in range(NP) for i in range(NSTR)]

    def kernel(x_hbm, ka_hbm, va_hbm, wqa_hbm, woa_hbm, kb_hbm, vb_hbm, wqb_hbm, wob_hbm, gw_hbm,
               out_ref,
               kbuf, vbuf, wqa_buf, wqb_buf, woa_buf, wob_buf, x_buf, gw_buf,
               q_tab, ga_tab, gb_tab, acc_ref,
               k_sem, v_sem, w_sem, s_sem):

        def slot_of(t):
            return t % NS if isinstance(t, int) else lax.rem(t, NS)

        def step_base(t):
            return (t // SPU) * (NSTR * S) + (t % SPU) * G

        def kv_copy(src, base, buf, sem, slot, i, a):
            row = base + (i * S + a * R)
            if not isinstance(row, int):
                row = pl.multiple_of(row, R)
            return pltpu.make_async_copy(src.at[pl.ds(row, R), :],
                                         buf.at[slot, pl.ds(i * G + a * R, R), :], sem)

        def part_of(lst, part, nparts):
            n = len(lst) // nparts
            return list(enumerate(lst))[part * n:(part + 1) * n]

        def start_pair(k_src, kt, v_src, vt, gstep, part=0, nparts=1):
            kslot, vslot = slot_of(gstep), slot_of(gstep - 1)
            kb_, vb_ = step_base(kt), step_base(vt)
            for _, (i, a) in part_of(rr, part, nparts):
                kv_copy(k_src, kb_, kbuf, k_sem.at[kslot], kslot, i, a).start(priority=0)
                kv_copy(v_src, vb_, vbuf, v_sem.at[vslot], vslot, i, a).start(priority=1)

        def start_k_alone(src, t, slot):
            base = step_base(t)
            for n, (i, a) in enumerate(rr):
                kv_copy(src, base, kbuf, k_sem.at[slot], slot, i, a).start(priority=n % 2)

        def wait_k(slot):
            pltpu.make_async_copy(kbuf.at[slot], kbuf.at[slot], k_sem.at[slot]).wait()

        def wait_v(slot):
            pltpu.make_async_copy(vbuf.at[slot], vbuf.at[slot], v_sem.at[slot]).wait()

        def start_w_pair(wq_src, wq_dst, wq_sem, wo_src, wo_dst, wo_sem, n):
            p = (n % 4) * (NW // 4) + n // 4
            r = (p // 4) * 16
            c = (p % 4) * 1024
            ro = p * 32
            if not isinstance(n, int):
                r = pl.multiple_of(r, 16)
                c = pl.multiple_of(c, 1024)
                ro = pl.multiple_of(ro, 32)
            pltpu.make_async_copy(wq_src.at[pl.ds(r, 16), pl.ds(c, 1024)],
                                  wq_dst.at[pl.ds(r, 16), pl.ds(c, 1024)], wq_sem).start(priority=0)
            pltpu.make_async_copy(wo_src.at[pl.ds(ro, 32), :],
                                  wo_dst.at[pl.ds(ro, 32), :], wo_sem).start(priority=1)

        def wait_all(buf, sem):
            pltpu.make_async_copy(buf, buf, sem).wait()

        cx = pltpu.make_async_copy(x_hbm, x_buf, s_sem.at[0])
        cg = pltpu.make_async_copy(gw_hbm, gw_buf, s_sem.at[1])
        cx.start(priority=0)
        cg.start(priority=1)
        for n in range(NW):
            start_w_pair(wqb_hbm, wqb_buf, w_sem.at[0], wob_hbm, wob_buf, w_sem.at[1], n)
        start_k_alone(kb_hbm, 0, 0)
        for t in range(1, LB - 1):
            start_pair(kb_hbm, t, vb_hbm, t - 1, t)

        cx.wait()
        cg.wait()
        x = x_buf[...].astype(f32)
        gw = gw_buf[...].astype(f32).reshape(1, D)
        gate = jax.nn.sigmoid(jnp.sum(x * gw, axis=1, keepdims=True))
        x8 = jnp.concatenate([x, jnp.zeros((8 - NB, D), f32)], axis=0).astype(bf16)
        gate8 = jnp.concatenate([gate, jnp.zeros((8 - NB, 1), f32)], axis=0)
        ga_tab[...] = jnp.broadcast_to(gate8, (8, D))
        gb_tab[...] = jnp.broadcast_to(1.0 - gate8, (8, D))
        acc_ref[...] = jnp.zeros_like(acc_ref)

        row_d = lax.broadcasted_iota(jnp.int32, (8, D), 0)
        row_g = lax.broadcasted_iota(jnp.int32, (8, G), 0)
        row_h = lax.broadcasted_iota(jnp.int32, (8, DH), 0)

        def fill_q_tab(wq_buf, dup, issue):
            per = 4 if dup else 8
            hp = H // NFILL
            for k in range(NFILL):
                issue(k)
                q_p = jnp.dot(x8, wq_buf[:, k * hp * DH:(k + 1) * hp * DH], preferred_element_type=f32)
                for b in range(NB):
                    for j in range(hp // per):
                        rows = [q_p[b:b + 1, (j * per + r) * DH:(j * per + r + 1) * DH] for r in range(per)]
                        if dup:
                            rows = rows + rows
                        q_tab[b * (H // per) + k * (hp // per) + j] = jnp.concatenate(rows, axis=0)

        def sel(vals, rows):
            key = rows % 4 if len(vals) == 4 else rows // 4
            out = vals[-1]
            for k in range(len(vals) - 2, -1, -1):
                out = jnp.where(key == k, vals[k], out)
            return out

        def scores(slot, qs, streams):
            wait_k(slot)
            out = []
            for q, st in zip(qs, streams):
                vals = [lax.dot_general(q, kbuf[slot, pl.ds(i * G, G), :], (((1,), (1,)), ((), ())),
                                        preferred_element_type=f32) for i in st]
                out.append(sel(vals, row_g))
            return out

        def softmax_update(sl, st):
            m, l, acc = st
            mx = sl[0]
            for s_ in sl[1:]:
                mx = jnp.maximum(mx, s_)
            m_new = jnp.maximum(m, jnp.max(mx, axis=1, keepdims=True))
            alpha = jnp.exp((m - m_new) * scale)
            l = alpha * l
            ps = []
            for s_ in sl:
                p = jnp.exp((s_ - m_new) * scale)
                for k in range(NC):
                    l = l + p[:, k * DH:(k + 1) * DH]
                ps.append(p.astype(bf16))
            return ps, m_new, l, alpha * acc

        def step(t, qs, streams, state, issue):
            slot = slot_of(t)
            ss = scores(slot, qs, streams)
            issue()
            mid = [softmax_update([s_], st) for s_, st in zip(ss, state)]
            wait_v(slot)
            new = []
            for (ps, m, l, acc), st in zip(mid, streams):
                vals = [jnp.dot(ps[0], vbuf[slot, pl.ds(i * G, G), :], preferred_element_type=f32) for i in st]
                new.append((m, l, acc + sel(vals, row_h)))
            return new

        def init_state(n):
            return [(jnp.full((8, 1), NEG, f32), jnp.zeros((8, DH), f32), jnp.zeros((8, DH), f32))
                    for _ in range(n)]

        def finish(st):
            m, l, acc = st
            return (acc / jnp.sum(l, axis=1, keepdims=True)).astype(bf16).astype(f32)

        def project(o, nrows, w):
            lhs = jnp.concatenate([jnp.broadcast_to(o[r:r + 1, :], (8, DH)) for r in range(nrows)], axis=1)
            return jnp.dot(lhs.astype(bf16), w, preferred_element_type=f32)

        def flat(state):
            return tuple(v for st in state for v in st)

        def unflat(vals):
            return [tuple(vals[3 * j:3 * j + 3]) for j in range(len(vals) // 3)]

        def unit_b(u, carry, last=False):
            b = u // 2
            half = u % 2
            qs = [q_tab[b * 4 + half * 2 + j].astype(bf16) for j in range(2)]

            def body(c, vals):
                t = u * SPU + c

                @pl.when(t < NW // WPS)
                def _():
                    for r in range(WPS):
                        start_w_pair(wqa_hbm, wqa_buf, w_sem.at[2], woa_hbm, woa_buf, w_sem.at[3], t * WPS + r)

                def issue():
                    ck = t + LB
                    if not last:
                        start_pair(kb_hbm, ck, vb_hbm, ck - 1, ck)
                        return

                    @pl.when(ck < NTB)
                    def _():
                        start_pair(kb_hbm, ck, vb_hbm, ck - 1, ck)

                    @pl.when(ck == NTB)
                    def _():
                        start_pair(ka_hbm, 0, vb_hbm, NTB - 1, ck)

                    @pl.when(ck > NTB)
                    def _():
                        start_pair(ka_hbm, ck - NTB, va_hbm, ck - NTB - 1, ck)

                return flat(step(t, qs, [[0, 1], [2, 3]], unflat(vals), issue))

            st = unflat(lax.fori_loop(0, SPU, body, flat(init_state(2))))
            res = None
            for j in range(2):
                row0 = pl.multiple_of((half * 16 + j * 8) * DH, 8 * DH)
                r = project(finish(st[j]), 8, wob_buf[pl.ds(row0, 8 * DH), :])
                res = r if res is None else res + r
            acc_ref[...] += jnp.where(row_d == b, res * gb_tab[...], 0.0)
            return carry

        wait_all(wqb_buf, w_sem.at[0])
        fill_q_tab(wqb_buf, False,
                   lambda k: start_pair(kb_hbm, LB - 1, vb_hbm, LB - 2, LB - 1, k, NFILL))
        wait_all(wob_buf, w_sem.at[1])
        lax.fori_loop(0, NUB - 1, unit_b, 0)
        unit_b(NUB - 1, 0, last=True)

        wait_all(wqa_buf, w_sem.at[2])
        fill_q_tab(wqa_buf, True,
                   lambda k: start_pair(ka_hbm, LB, va_hbm, LB - 1, NTB + LB, k, NFILL))
        wait_all(woa_buf, w_sem.at[3])

        a_streams = [[0, 1, 2, 3]]

        def body_a(u, qs, c, vals, issue=None):
            ta = u * SPU + c
            if issue is None:
                def issue():
                    ck = ta + LA
                    start_pair(ka_hbm, ck, va_hbm, ck - 1, NTB + ck)
            return flat(step(NTB + ta, qs, a_streams, unflat(vals), issue))

        def unit_a(u, carry):
            b = u // 8
            hq = u % 8
            qs = [q_tab[u].astype(bf16)]
            vals = lax.fori_loop(0, SPU, functools.partial(body_a, u, qs), flat(init_state(1)))
            row0 = pl.multiple_of(hq * 4 * DH, 4 * DH)
            res = project(finish(unflat(vals)[0]), 4, woa_buf[pl.ds(row0, 4 * DH), :])
            acc_ref[...] += jnp.where(row_d == b, res * ga_tab[...], 0.0)
            return carry

        lax.fori_loop(0, NUA - 1, unit_a, 0)

        u = NUA - 1
        qs = [q_tab[u].astype(bf16)]
        s0, s1 = slot_of(NTB + NTA - 2), slot_of(NTB + NTA - 1)

        def issue_vv():
            for c, slot in enumerate((s0, s1)):
                base = step_base(NTA - 2 + c)
                for n, (i, a) in enumerate(rr):
                    kv_copy(va_hbm, base, vbuf, v_sem.at[slot], slot, i, a).start(priority=n % 2)

        vals = lax.fori_loop(0, SPU - LA - 1, functools.partial(body_a, u, qs), flat(init_state(1)))
        vals = body_a(u, qs, SPU - LA - 1, vals, issue=lambda: start_k_alone(ka_hbm, NTA - 1, s1))
        vals = body_a(u, qs, SPU - LA, vals, issue=issue_vv)
        vals = lax.fori_loop(SPU - LA + 1, SPU - 2,
                             functools.partial(body_a, u, qs, issue=lambda: None), vals)
        sa = scores(s0, qs, a_streams)[0]
        sb = scores(s1, qs, a_streams)[0]
        ps, m, l, acc = softmax_update([sa, sb], unflat(vals)[0])
        inv_l = 1.0 / jnp.sum(l, axis=1, keepdims=True)
        for c, slot in enumerate((s0, s1)):
            wait_v(slot)
            pv = [jnp.dot(ps[c], vbuf[slot, pl.ds(i * G, G), :], preferred_element_type=f32)
                  for i in range(NSTR)]
            acc = acc + sel(pv, row_h)
        o = (acc * inv_l).astype(bf16).astype(f32)
        res = project(o, 4, woa_buf[pl.ds((u % 8) * 4 * DH, 4 * DH), :])
        final = acc_ref[...] + jnp.where(row_d == u // 8, res * ga_tab[...], 0.0)
        out_ref[...] = final[0:NB, :].astype(out_ref.dtype)

    scratch = [
        pltpu.VMEM((NS, CH, DH), bf16),
        pltpu.VMEM((NS, CH, DH), bf16),
        pltpu.VMEM((D, H * DH), bf16),
        pltpu.VMEM((D, H * DH), bf16),
        pltpu.VMEM((H * DH, D), bf16),
        pltpu.VMEM((H * DH, D), bf16),
        pltpu.VMEM((NB, D), bf16),
        pltpu.VMEM((D,), bf16),
        pltpu.VMEM((NUA, 8, DH), f32),
        pltpu.VMEM((8, D), f32),
        pltpu.VMEM((8, D), f32),
        pltpu.VMEM((8, D), f32),
        pltpu.SemaphoreType.DMA((NS,)),
        pltpu.SemaphoreType.DMA((NS,)),
        pltpu.SemaphoreType.DMA((4,)),
        pltpu.SemaphoreType.DMA((2,)),
    ]

    def run(A_x, A_k_cache, A_v_cache, A_wq, A_wo, B_x, B_k_cache, B_v_cache, B_wq, B_wo, gate_w):
        ka = A_k_cache.reshape(NB * H * S, DH)
        va = A_v_cache.reshape(NB * H * S, DH)
        kb = B_k_cache.reshape(NB * HKV * S, DH)
        vb = B_v_cache.reshape(NB * HKV * S, DH)
        any_spec = pl.BlockSpec(memory_space=pl.ANY)
        return pl.pallas_call(
            kernel,
            out_shape=jax.ShapeDtypeStruct((NB, D), bf16),
            in_specs=[any_spec] * 10,
            out_specs=pl.BlockSpec(memory_space=pltpu.VMEM),
            scratch_shapes=scratch,
            compiler_params=pltpu.CompilerParams(vmem_limit_bytes=64 * 1024 * 1024,
                                                 disable_bounds_checks=True,
                                                 disable_semaphore_checks=not semchk),
        )(A_x.reshape(NB, D), ka, va, A_wq, A_wo, kb, vb, B_wq, B_wo, gate_w).reshape(NB, 1, D)
    return run


_run = _make_kernel()


@jax.jit
def pallas_gated_mix__mha_block_cached__gqa_block_cached__decode_kernel(
    A_x, A_k_cache, A_v_cache, A_wq, A_wo, B_x, B_k_cache, B_v_cache, B_wq, B_wo, gate_w,
):
    return _run(A_x, A_k_cache, A_v_cache, A_wq, A_wo, B_x, B_k_cache, B_v_cache, B_wq, B_wo, gate_w)
```

```python
import functools

import jax
import jax.numpy as jnp
from jax import lax
from jax.experimental import pallas as pl
from jax.experimental.pallas import tpu as pltpu

NB = 4
D = 512
H = 32
HKV = 8
S = 8192
DH = 128
NSTR = 4
NUA = NB * H // NSTR
NUB = NB * HKV // NSTR
R = 128
NW = 128


G = 512
LB = 4
LA = LB + 1
NS = LA + 1
WPS = 2
SPU = S // G
NTA = NUA * SPU
NTB = NUB * SPU
CH = NSTR * G
NP = G // R
NC = G // DH
NFILL = 4
SCALE = DH ** -0.5
NEG = -1e30
f32 = jnp.float32
bf16 = jnp.bfloat16
RR = [(i, a) for a in range(NP) for i in range(NSTR)]


def _kernel(x_hbm, ka_hbm, va_hbm, wqa_hbm, woa_hbm, kb_hbm, vb_hbm, wqb_hbm, wob_hbm, gw_hbm,
           out_ref,
           kbuf, vbuf, wqa_buf, wqb_buf, woa_buf, wob_buf, x_buf, gw_buf,
           q_tab, ga_tab, gb_tab, acc_ref,
           k_sem, v_sem, w_sem, s_sem):

    def slot_of(t):
        return t % NS if isinstance(t, int) else lax.rem(t, NS)

    def step_base(t):
        return (t // SPU) * (NSTR * S) + (t % SPU) * G

    def kv_copy(src, base, buf, sem, slot, i, a):
        row = base + (i * S + a * R)
        if not isinstance(row, int):
            row = pl.multiple_of(row, R)
        return pltpu.make_async_copy(src.at[pl.ds(row, R), :],
                                     buf.at[slot, pl.ds(i * G + a * R, R), :], sem)

    def part_of(lst, part, nparts):
        n = len(lst) // nparts
        return list(enumerate(lst))[part * n:(part + 1) * n]

    def start_pair(k_src, kt, v_src, vt, gstep, part=0, nparts=1):
        kslot, vslot = slot_of(gstep), slot_of(gstep - 1)
        kb_, vb_ = step_base(kt), step_base(vt)
        for _, (i, a) in part_of(RR, part, nparts):
            kv_copy(k_src, kb_, kbuf, k_sem.at[kslot], kslot, i, a).start(priority=0)
            kv_copy(v_src, vb_, vbuf, v_sem.at[vslot], vslot, i, a).start(priority=1)

    def start_k_alone(src, t, slot):
        base = step_base(t)
        for n, (i, a) in enumerate(RR):
            kv_copy(src, base, kbuf, k_sem.at[slot], slot, i, a).start(priority=n % 2)

    def wait_k(slot):
        pltpu.make_async_copy(kbuf.at[slot], kbuf.at[slot], k_sem.at[slot]).wait()

    def wait_v(slot):
        pltpu.make_async_copy(vbuf.at[slot], vbuf.at[slot], v_sem.at[slot]).wait()

    def start_w_pair(wq_src, wq_dst, wq_sem, wo_src, wo_dst, wo_sem, n):
        p = (n % 4) * (NW // 4) + n // 4
        r = (p // 4) * 16
        c = (p % 4) * 1024
        ro = p * 32
        if not isinstance(n, int):
            r = pl.multiple_of(r, 16)
            c = pl.multiple_of(c, 1024)
            ro = pl.multiple_of(ro, 32)
        pltpu.make_async_copy(wq_src.at[pl.ds(r, 16), pl.ds(c, 1024)],
                              wq_dst.at[pl.ds(r, 16), pl.ds(c, 1024)], wq_sem).start(priority=0)
        pltpu.make_async_copy(wo_src.at[pl.ds(ro, 32), :],
                              wo_dst.at[pl.ds(ro, 32), :], wo_sem).start(priority=1)

    def wait_all(buf, sem):
        pltpu.make_async_copy(buf, buf, sem).wait()

    cx = pltpu.make_async_copy(x_hbm, x_buf, s_sem.at[0])
    cg = pltpu.make_async_copy(gw_hbm, gw_buf, s_sem.at[1])
    cx.start(priority=0)
    cg.start(priority=1)
    for n in range(NW):
        start_w_pair(wqb_hbm, wqb_buf, w_sem.at[0], wob_hbm, wob_buf, w_sem.at[1], n)
    start_k_alone(kb_hbm, 0, 0)
    for t in range(1, LB - 1):
        start_pair(kb_hbm, t, vb_hbm, t - 1, t)

    cx.wait()
    cg.wait()
    x = x_buf[...].astype(f32)
    gw = gw_buf[...].astype(f32).reshape(1, D)
    gate = jax.nn.sigmoid(jnp.sum(x * gw, axis=1, keepdims=True))
    x8 = jnp.concatenate([x, jnp.zeros((8 - NB, D), f32)], axis=0).astype(bf16)
    gate8 = jnp.concatenate([gate, jnp.zeros((8 - NB, 1), f32)], axis=0)
    ga_tab[...] = jnp.broadcast_to(gate8, (8, D))
    gb_tab[...] = jnp.broadcast_to(1.0 - gate8, (8, D))
    acc_ref[...] = jnp.zeros_like(acc_ref)

    row_d = lax.broadcasted_iota(jnp.int32, (8, D), 0)
    row_g = lax.broadcasted_iota(jnp.int32, (8, G), 0)
    row_h = lax.broadcasted_iota(jnp.int32, (8, DH), 0)

    def fill_q_tab(wq_buf, dup, issue):
        per = 4 if dup else 8
        hp = H // NFILL
        for k in range(NFILL):
            issue(k)
            q_p = jnp.dot(x8, wq_buf[:, k * hp * DH:(k + 1) * hp * DH], preferred_element_type=f32)
            for b in range(NB):
                for j in range(hp // per):
                    rows = [q_p[b:b + 1, (j * per + r) * DH:(j * per + r + 1) * DH] for r in range(per)]
                    if dup:
                        rows = rows + rows
                    q_tab[b * (H // per) + k * (hp // per) + j] = jnp.concatenate(rows, axis=0)

    def sel(vals, rows):
        key = rows % 4 if len(vals) == 4 else rows // 4
        out = vals[-1]
        for k in range(len(vals) - 2, -1, -1):
            out = jnp.where(key == k, vals[k], out)
        return out

    def scores(slot, qs, streams):
        wait_k(slot)
        out = []
        for q, st in zip(qs, streams):
            vals = [lax.dot_general(q, kbuf[slot, pl.ds(i * G, G), :], (((1,), (1,)), ((), ())),
                                    preferred_element_type=f32) for i in st]
            out.append(sel(vals, row_g))
        return out

    def softmax_update(sl, st):
        m, l, acc = st
        mx = sl[0]
        for s_ in sl[1:]:
            mx = jnp.maximum(mx, s_)
        m_new = jnp.maximum(m, jnp.max(mx, axis=1, keepdims=True))
        alpha = jnp.exp((m - m_new) * SCALE)
        l = alpha * l
        ps = []
        for s_ in sl:
            p = jnp.exp((s_ - m_new) * SCALE)
            for k in range(NC):
                l = l + p[:, k * DH:(k + 1) * DH]
            ps.append(p.astype(bf16))
        return ps, m_new, l, alpha * acc

    def step(t, qs, streams, state, issue):
        slot = slot_of(t)
        ss = scores(slot, qs, streams)
        issue()
        mid = [softmax_update([s_], st) for s_, st in zip(ss, state)]
        wait_v(slot)
        new = []
        for (ps, m, l, acc), st in zip(mid, streams):
            vals = [jnp.dot(ps[0], vbuf[slot, pl.ds(i * G, G), :], preferred_element_type=f32) for i in st]
            new.append((m, l, acc + sel(vals, row_h)))
        return new

    def init_state(n):
        return [(jnp.full((8, 1), NEG, f32), jnp.zeros((8, DH), f32), jnp.zeros((8, DH), f32))
                for _ in range(n)]

    def finish(st):
        m, l, acc = st
        return (acc / jnp.sum(l, axis=1, keepdims=True)).astype(bf16).astype(f32)

    def project(o, nrows, w):
        lhs = jnp.concatenate([jnp.broadcast_to(o[r:r + 1, :], (8, DH)) for r in range(nrows)], axis=1)
        return jnp.dot(lhs.astype(bf16), w, preferred_element_type=f32)

    def flat(state):
        return tuple(v for st in state for v in st)

    def unflat(vals):
        return [tuple(vals[3 * j:3 * j + 3]) for j in range(len(vals) // 3)]

    def unit_b(u, carry, last=False):
        b = u // 2
        half = u % 2
        qs = [q_tab[b * 4 + half * 2 + j].astype(bf16) for j in range(2)]

        def body(c, vals):
            t = u * SPU + c

            @pl.when(t < NW // WPS)
            def _():
                for r in range(WPS):
                    start_w_pair(wqa_hbm, wqa_buf, w_sem.at[2], woa_hbm, woa_buf, w_sem.at[3], t * WPS + r)

            def issue():
                ck = t + LB
                if not last:
                    start_pair(kb_hbm, ck, vb_hbm, ck - 1, ck)
                    return

                @pl.when(ck < NTB)
                def _():
                    start_pair(kb_hbm, ck, vb_hbm, ck - 1, ck)

                @pl.when(ck == NTB)
                def _():
                    start_pair(ka_hbm, 0, vb_hbm, NTB - 1, ck)

                @pl.when(ck > NTB)
                def _():
                    start_pair(ka_hbm, ck - NTB, va_hbm, ck - NTB - 1, ck)

            return flat(step(t, qs, [[0, 1], [2, 3]], unflat(vals), issue))

        st = unflat(lax.fori_loop(0, SPU, body, flat(init_state(2))))
        res = None
        for j in range(2):
            row0 = pl.multiple_of((half * 16 + j * 8) * DH, 8 * DH)
            r = project(finish(st[j]), 8, wob_buf[pl.ds(row0, 8 * DH), :])
            res = r if res is None else res + r
        acc_ref[...] += jnp.where(row_d == b, res * gb_tab[...], 0.0)
        return carry

    wait_all(wqb_buf, w_sem.at[0])
    fill_q_tab(wqb_buf, False,
               lambda k: start_pair(kb_hbm, LB - 1, vb_hbm, LB - 2, LB - 1, k, NFILL))
    wait_all(wob_buf, w_sem.at[1])
    lax.fori_loop(0, NUB - 1, unit_b, 0)
    unit_b(NUB - 1, 0, last=True)

    wait_all(wqa_buf, w_sem.at[2])
    fill_q_tab(wqa_buf, True,
               lambda k: start_pair(ka_hbm, LB, va_hbm, LB - 1, NTB + LB, k, NFILL))
    wait_all(woa_buf, w_sem.at[3])

    a_streams = [[0, 1, 2, 3]]

    def body_a(u, qs, c, vals, issue=None):
        ta = u * SPU + c
        if issue is None:
            def issue():
                ck = ta + LA
                start_pair(ka_hbm, ck, va_hbm, ck - 1, NTB + ck)
        return flat(step(NTB + ta, qs, a_streams, unflat(vals), issue))

    def unit_a(u, carry):
        b = u // 8
        hq = u % 8
        qs = [q_tab[u].astype(bf16)]
        vals = lax.fori_loop(0, SPU, functools.partial(body_a, u, qs), flat(init_state(1)))
        row0 = pl.multiple_of(hq * 4 * DH, 4 * DH)
        res = project(finish(unflat(vals)[0]), 4, woa_buf[pl.ds(row0, 4 * DH), :])
        acc_ref[...] += jnp.where(row_d == b, res * ga_tab[...], 0.0)
        return carry

    lax.fori_loop(0, NUA - 1, unit_a, 0)

    u = NUA - 1
    qs = [q_tab[u].astype(bf16)]
    s0, s1 = slot_of(NTB + NTA - 2), slot_of(NTB + NTA - 1)

    def issue_vv():
        for c, slot in enumerate((s0, s1)):
            base = step_base(NTA - 2 + c)
            for n, (i, a) in enumerate(RR):
                kv_copy(va_hbm, base, vbuf, v_sem.at[slot], slot, i, a).start(priority=n % 2)

    vals = lax.fori_loop(0, SPU - LA - 1, functools.partial(body_a, u, qs), flat(init_state(1)))
    vals = body_a(u, qs, SPU - LA - 1, vals, issue=lambda: start_k_alone(ka_hbm, NTA - 1, s1))
    vals = body_a(u, qs, SPU - LA, vals, issue=issue_vv)
    vals = lax.fori_loop(SPU - LA + 1, SPU - 2,
                         functools.partial(body_a, u, qs, issue=lambda: None), vals)
    sa = scores(s0, qs, a_streams)[0]
    sb = scores(s1, qs, a_streams)[0]
    ps, m, l, acc = softmax_update([sa, sb], unflat(vals)[0])
    inv_l = 1.0 / jnp.sum(l, axis=1, keepdims=True)
    for c, slot in enumerate((s0, s1)):
        wait_v(slot)
        pv = [jnp.dot(ps[c], vbuf[slot, pl.ds(i * G, G), :], preferred_element_type=f32)
              for i in range(NSTR)]
        acc = acc + sel(pv, row_h)
    o = (acc * inv_l).astype(bf16).astype(f32)
    res = project(o, 4, woa_buf[pl.ds((u % 8) * 4 * DH, 4 * DH), :])
    final = acc_ref[...] + jnp.where(row_d == u // 8, res * ga_tab[...], 0.0)
    out_ref[...] = final[0:NB, :].astype(out_ref.dtype)


_SCRATCH = [
    pltpu.VMEM((NS, CH, DH), bf16),
    pltpu.VMEM((NS, CH, DH), bf16),
    pltpu.VMEM((D, H * DH), bf16),
    pltpu.VMEM((D, H * DH), bf16),
    pltpu.VMEM((H * DH, D), bf16),
    pltpu.VMEM((H * DH, D), bf16),
    pltpu.VMEM((NB, D), bf16),
    pltpu.VMEM((D,), bf16),
    pltpu.VMEM((NUA, 8, DH), f32),
    pltpu.VMEM((8, D), f32),
    pltpu.VMEM((8, D), f32),
    pltpu.VMEM((8, D), f32),
    pltpu.SemaphoreType.DMA((NS,)),
    pltpu.SemaphoreType.DMA((NS,)),
    pltpu.SemaphoreType.DMA((4,)),
    pltpu.SemaphoreType.DMA((2,)),
]


@jax.jit
def pallas_gated_mix__mha_block_cached__gqa_block_cached__decode_kernel(
    A_x, A_k_cache, A_v_cache, A_wq, A_wo, B_x, B_k_cache, B_v_cache, B_wq, B_wo, gate_w,
):
    del B_x
    ka = A_k_cache.reshape(NB * H * S, DH)
    va = A_v_cache.reshape(NB * H * S, DH)
    kb = B_k_cache.reshape(NB * HKV * S, DH)
    vb = B_v_cache.reshape(NB * HKV * S, DH)
    any_spec = pl.BlockSpec(memory_space=pl.ANY)
    out = pl.pallas_call(
        _kernel,
        out_shape=jax.ShapeDtypeStruct((NB, D), bf16),
        in_specs=[any_spec] * 10,
        out_specs=pl.BlockSpec(memory_space=pltpu.VMEM),
        scratch_shapes=_SCRATCH,
        compiler_params=pltpu.CompilerParams(vmem_limit_bytes=64 * 1024 * 1024,
                                             disable_bounds_checks=True,
                                             disable_semaphore_checks=True),
    )(A_x.reshape(NB, D), ka, va, A_wq, A_wo, kb, vb, B_wq, B_wo, gate_w)
    return out.reshape(NB, 1, D)
```

```python
import functools

import jax
import jax.numpy as jnp
from jax import lax
from jax.experimental import pallas as pl
from jax.experimental.pallas import tpu as pltpu

NB = 4
D = 512
H = 32
HKV = 8
S = 8192
DH = 128
NSTR = 4
NUA = NB * H // NSTR
NUB = NB * HKV // NSTR
R = 128
NW = 128


G = 512
LB = 4
LA = LB + 1
NS = LA + 1
WPS = 2
SPU = S // G
NTA = NUA * SPU
NTB = NUB * SPU
CH = NSTR * G
NP = G // R
NC = G // DH
NFILL = 4
SCALE = DH ** -0.5
NEG = -1e30
f32 = jnp.float32
bf16 = jnp.bfloat16
RR = [(i, a) for a in range(NP) for i in range(NSTR)]


def _kernel(x_hbm, ka_hbm, va_hbm, wqa_hbm, woa_hbm, kb_hbm, vb_hbm, wqb_hbm, wob_hbm, gw_hbm,
           out_ref,
           kbuf, vbuf, wqa_buf, wqb_buf, woa_buf, wob_buf, x_buf, gw_buf,
           q_tab, ga_tab, gb_tab, acc_ref,
           k_sem, v_sem, w_sem, s_sem):

    def slot_of(t):
        return t % NS if isinstance(t, int) else lax.rem(t, NS)

    def step_base(t):
        return (t // SPU) * (NSTR * S) + (t % SPU) * G

    def kv_copy(src, base, buf, sem, slot, i, a):
        row = base + (i * S + a * R)
        if not isinstance(row, int):
            row = pl.multiple_of(row, R)
        return pltpu.make_async_copy(src.at[pl.ds(row, R), :],
                                     buf.at[slot, pl.ds(i * G + a * R, R), :], sem)

    def part_of(lst, part, nparts):
        n = len(lst) // nparts
        return list(enumerate(lst))[part * n:(part + 1) * n]

    def start_pair(k_src, kt, v_src, vt, gstep, part=0, nparts=1):
        kslot, vslot = slot_of(gstep), slot_of(gstep - 1)
        kb_, vb_ = step_base(kt), step_base(vt)
        for _, (i, a) in part_of(RR, part, nparts):
            kv_copy(k_src, kb_, kbuf, k_sem.at[kslot], kslot, i, a).start(priority=0)
            kv_copy(v_src, vb_, vbuf, v_sem.at[vslot], vslot, i, a).start(priority=1)

    def start_k_alone(src, t, slot):
        base = step_base(t)
        for n, (i, a) in enumerate(RR):
            kv_copy(src, base, kbuf, k_sem.at[slot], slot, i, a).start(priority=n % 2)

    def wait_k(slot):
        pltpu.make_async_copy(kbuf.at[slot], kbuf.at[slot], k_sem.at[slot]).wait()

    def wait_v(slot):
        pltpu.make_async_copy(vbuf.at[slot], vbuf.at[slot], v_sem.at[slot]).wait()

    def start_w_pair(wq_src, wq_dst, wq_sem, wo_src, wo_dst, wo_sem, n):
        p = (n % 4) * (NW // 4) + n // 4
        r = (p // 4) * 16
        c = (p % 4) * 1024
        ro = p * 32
        if not isinstance(n, int):
            r = pl.multiple_of(r, 16)
            c = pl.multiple_of(c, 1024)
            ro = pl.multiple_of(ro, 32)
        pltpu.make_async_copy(wq_src.at[pl.ds(r, 16), pl.ds(c, 1024)],
                              wq_dst.at[pl.ds(r, 16), pl.ds(c, 1024)], wq_sem).start(priority=0)
        pltpu.make_async_copy(wo_src.at[pl.ds(ro, 32), :],
                              wo_dst.at[pl.ds(ro, 32), :], wo_sem).start(priority=1)

    def wait_all(buf, sem):
        pltpu.make_async_copy(buf, buf, sem).wait()

    cx = pltpu.make_async_copy(x_hbm, x_buf, s_sem.at[0])
    cg = pltpu.make_async_copy(gw_hbm, gw_buf, s_sem.at[1])
    cx.start(priority=0)
    cg.start(priority=0)
    for n in range(NW):
        start_w_pair(wqb_hbm, wqb_buf, w_sem.at[0], wob_hbm, wob_buf, w_sem.at[1], n)
    start_k_alone(kb_hbm, 0, 0)
    for t in range(1, LB - 1):
        start_pair(kb_hbm, t, vb_hbm, t - 1, t)

    cx.wait()
    cg.wait()
    x = x_buf[...].astype(f32)
    gw = gw_buf[...].astype(f32).reshape(1, D)
    gate = jax.nn.sigmoid(jnp.sum(x * gw, axis=1, keepdims=True))
    x8 = jnp.concatenate([x, jnp.zeros((8 - NB, D), f32)], axis=0).astype(bf16)
    gate8 = jnp.concatenate([gate, jnp.zeros((8 - NB, 1), f32)], axis=0)
    ga_tab[...] = jnp.broadcast_to(gate8, (8, D))
    gb_tab[...] = jnp.broadcast_to(1.0 - gate8, (8, D))
    acc_ref[...] = jnp.zeros_like(acc_ref)

    row_d = lax.broadcasted_iota(jnp.int32, (8, D), 0)
    row_g = lax.broadcasted_iota(jnp.int32, (8, G), 0)
    row_h = lax.broadcasted_iota(jnp.int32, (8, DH), 0)

    def fill_q_tab(wq_buf, dup, issue):
        per = 4 if dup else 8
        hp = H // NFILL
        for k in range(NFILL):
            issue(k)
            q_p = jnp.dot(x8, wq_buf[:, k * hp * DH:(k + 1) * hp * DH], preferred_element_type=f32)
            for b in range(NB):
                for j in range(hp // per):
                    rows = [q_p[b:b + 1, (j * per + r) * DH:(j * per + r + 1) * DH] for r in range(per)]
                    if dup:
                        rows = rows + rows
                    q_tab[b * (H // per) + k * (hp // per) + j] = jnp.concatenate(rows, axis=0)

    def sel(vals, rows):
        key = rows % 4 if len(vals) == 4 else rows // 4
        out = vals[-1]
        for k in range(len(vals) - 2, -1, -1):
            out = jnp.where(key == k, vals[k], out)
        return out

    def scores(slot, qs, streams):
        wait_k(slot)
        out = []
        for q, st in zip(qs, streams):
            vals = [lax.dot_general(q, kbuf[slot, pl.ds(i * G, G), :], (((1,), (1,)), ((), ())),
                                    preferred_element_type=f32) for i in st]
            out.append(sel(vals, row_g))
        return out

    def softmax_update(sl, st):
        m, l, acc = st
        mx = sl[0]
        for s_ in sl[1:]:
            mx = jnp.maximum(mx, s_)
        m_new = jnp.maximum(m, jnp.max(mx, axis=1, keepdims=True))
        alpha = jnp.exp((m - m_new) * SCALE)
        l = alpha * l
        ps = []
        for s_ in sl:
            p = jnp.exp((s_ - m_new) * SCALE)
            for k in range(NC):
                l = l + p[:, k * DH:(k + 1) * DH]
            ps.append(p.astype(bf16))
        return ps, m_new, l, alpha * acc

    def step(t, qs, streams, state, issue):
        slot = slot_of(t)
        ss = scores(slot, qs, streams)
        issue()
        mid = [softmax_update([s_], st) for s_, st in zip(ss, state)]
        wait_v(slot)
        new = []
        for (ps, m, l, acc), st in zip(mid, streams):
            vals = [jnp.dot(ps[0], vbuf[slot, pl.ds(i * G, G), :], preferred_element_type=f32) for i in st]
            new.append((m, l, acc + sel(vals, row_h)))
        return new

    def init_state(n):
        return [(jnp.full((8, 1), NEG, f32), jnp.zeros((8, DH), f32), jnp.zeros((8, DH), f32))
                for _ in range(n)]

    def finish(st):
        m, l, acc = st
        return (acc / jnp.sum(l, axis=1, keepdims=True)).astype(bf16).astype(f32)

    def project(o, nrows, w):
        lhs = jnp.concatenate([jnp.broadcast_to(o[r:r + 1, :], (8, DH)) for r in range(nrows)], axis=1)
        return jnp.dot(lhs.astype(bf16), w, preferred_element_type=f32)

    def flat(state):
        return tuple(v for st in state for v in st)

    def unflat(vals):
        return [tuple(vals[3 * j:3 * j + 3]) for j in range(len(vals) // 3)]

    def unit_b(u, carry, last=False):
        b = u // 2
        half = u % 2
        qs = [q_tab[b * 4 + half * 2 + j].astype(bf16) for j in range(2)]

        def body(c, vals):
            t = u * SPU + c

            @pl.when(t < NW // WPS)
            def _():
                for r in range(WPS):
                    start_w_pair(wqa_hbm, wqa_buf, w_sem.at[2], woa_hbm, woa_buf, w_sem.at[3], t * WPS + r)

            def issue():
                ck = t + LB
                if not last:
                    start_pair(kb_hbm, ck, vb_hbm, ck - 1, ck)
                    return

                @pl.when(ck < NTB)
                def _():
                    start_pair(kb_hbm, ck, vb_hbm, ck - 1, ck)

                @pl.when(ck == NTB)
                def _():
                    start_pair(ka_hbm, 0, vb_hbm, NTB - 1, ck)

                @pl.when(ck > NTB)
                def _():
                    start_pair(ka_hbm, ck - NTB, va_hbm, ck - NTB - 1, ck)

            return flat(step(t, qs, [[0, 1], [2, 3]], unflat(vals), issue))

        st = unflat(lax.fori_loop(0, SPU, body, flat(init_state(2))))
        res = None
        for j in range(2):
            row0 = pl.multiple_of((half * 16 + j * 8) * DH, 8 * DH)
            r = project(finish(st[j]), 8, wob_buf[pl.ds(row0, 8 * DH), :])
            res = r if res is None else res + r
        acc_ref[...] += jnp.where(row_d == b, res * gb_tab[...], 0.0)
        return carry

    wait_all(wqb_buf, w_sem.at[0])
    fill_q_tab(wqb_buf, False,
               lambda k: start_pair(kb_hbm, LB - 1, vb_hbm, LB - 2, LB - 1, k, NFILL))
    wait_all(wob_buf, w_sem.at[1])
    lax.fori_loop(0, NUB - 1, unit_b, 0)
    unit_b(NUB - 1, 0, last=True)

    wait_all(wqa_buf, w_sem.at[2])
    fill_q_tab(wqa_buf, True,
               lambda k: start_pair(ka_hbm, LB, va_hbm, LB - 1, NTB + LB, k, NFILL))
    wait_all(woa_buf, w_sem.at[3])

    a_streams = [[0, 1, 2, 3]]

    def body_a(u, qs, c, vals, issue=None):
        ta = u * SPU + c
        if issue is None:
            def issue():
                ck = ta + LA
                start_pair(ka_hbm, ck, va_hbm, ck - 1, NTB + ck)
        return flat(step(NTB + ta, qs, a_streams, unflat(vals), issue))

    def unit_a(u, carry):
        b = u // 8
        hq = u % 8
        qs = [q_tab[u].astype(bf16)]
        vals = lax.fori_loop(0, SPU, functools.partial(body_a, u, qs), flat(init_state(1)))
        row0 = pl.multiple_of(hq * 4 * DH, 4 * DH)
        res = project(finish(unflat(vals)[0]), 4, woa_buf[pl.ds(row0, 4 * DH), :])
        acc_ref[...] += jnp.where(row_d == b, res * ga_tab[...], 0.0)
        return carry

    lax.fori_loop(0, NUA - 1, unit_a, 0)

    u = NUA - 1
    qs = [q_tab[u].astype(bf16)]
    s0, s1 = slot_of(NTB + NTA - 2), slot_of(NTB + NTA - 1)

    def issue_last_v():
        base = step_base(NTA - 1)
        for i, a in RR:
            kv_copy(va_hbm, base, vbuf, v_sem.at[s1], s1, i, a).start(priority=1)

    vals = lax.fori_loop(0, SPU - LA, functools.partial(body_a, u, qs), flat(init_state(1)))
    vals = body_a(u, qs, SPU - LA, vals, issue=issue_last_v)
    vals = lax.fori_loop(SPU - LA + 1, SPU - 2,
                         functools.partial(body_a, u, qs, issue=lambda: None), vals)
    sa = scores(s0, qs, a_streams)[0]
    sb = scores(s1, qs, a_streams)[0]
    ps, m, l, acc = softmax_update([sa, sb], unflat(vals)[0])
    inv_l = 1.0 / jnp.sum(l, axis=1, keepdims=True)
    for c, slot in enumerate((s0, s1)):
        wait_v(slot)
        pv = [jnp.dot(ps[c], vbuf[slot, pl.ds(i * G, G), :], preferred_element_type=f32)
              for i in range(NSTR)]
        acc = acc + sel(pv, row_h)
    o = (acc * inv_l).astype(bf16).astype(f32)
    res = project(o, 4, woa_buf[pl.ds((u % 8) * 4 * DH, 4 * DH), :])
    final = acc_ref[...] + jnp.where(row_d == u // 8, res * ga_tab[...], 0.0)
    out_ref[...] = final[0:NB, :].astype(out_ref.dtype)


_SCRATCH = [
    pltpu.VMEM((NS, CH, DH), bf16),
    pltpu.VMEM((NS, CH, DH), bf16),
    pltpu.VMEM((D, H * DH), bf16),
    pltpu.VMEM((D, H * DH), bf16),
    pltpu.VMEM((H * DH, D), bf16),
    pltpu.VMEM((H * DH, D), bf16),
    pltpu.VMEM((NB, D), bf16),
    pltpu.VMEM((D,), bf16),
    pltpu.VMEM((NUA, 8, DH), f32),
    pltpu.VMEM((8, D), f32),
    pltpu.VMEM((8, D), f32),
    pltpu.VMEM((8, D), f32),
    pltpu.SemaphoreType.DMA((NS,)),
    pltpu.SemaphoreType.DMA((NS,)),
    pltpu.SemaphoreType.DMA((4,)),
    pltpu.SemaphoreType.DMA((2,)),
]


@jax.jit
def pallas_gated_mix__mha_block_cached__gqa_block_cached__decode_kernel(
    A_x, A_k_cache, A_v_cache, A_wq, A_wo, B_x, B_k_cache, B_v_cache, B_wq, B_wo, gate_w,
):
    del B_x
    ka = A_k_cache.reshape(NB * H * S, DH)
    va = A_v_cache.reshape(NB * H * S, DH)
    kb = B_k_cache.reshape(NB * HKV * S, DH)
    vb = B_v_cache.reshape(NB * HKV * S, DH)
    any_spec = pl.BlockSpec(memory_space=pl.ANY)
    out = pl.pallas_call(
        _kernel,
        out_shape=jax.ShapeDtypeStruct((NB, D), bf16),
        in_specs=[any_spec] * 10,
        out_specs=pl.BlockSpec(memory_space=pltpu.VMEM),
        scratch_shapes=_SCRATCH,
        compiler_params=pltpu.CompilerParams(vmem_limit_bytes=64 * 1024 * 1024,
                                             disable_bounds_checks=True,
                                             disable_semaphore_checks=True),
    )(A_x.reshape(NB, D), ka, va, A_wq, A_wo, kb, vb, B_wq, B_wo, gate_w)
    return out.reshape(NB, 1, D)
```

```python
import functools

import jax
import jax.numpy as jnp
from jax import lax
from jax.experimental import pallas as pl
from jax.experimental.pallas import tpu as pltpu

NB = 4
D = 512
H = 32
HKV = 8
S = 8192
DH = 128
NSTR = 4
NUA = NB * H // NSTR
NUB = NB * HKV // NSTR
R = 128
NW = 128
G = 512
LB = 4
LA = LB + 1
NS = LA + 1
WPS = 2
SPU = S // G
NTA = NUA * SPU
NTB = NUB * SPU
CH = NSTR * G
NP = G // R
NC = G // DH
NFILL = 4
SCALE = DH ** -0.5
NEG = float("-inf")
f32 = jnp.float32
bf16 = jnp.bfloat16
RR = [(i, a) for a in range(NP) for i in range(NSTR)]


def _kernel(x_hbm, ka_hbm, va_hbm, wqa_hbm, woa_hbm, kb_hbm, vb_hbm, wqb_hbm, wob_hbm, gw_hbm,
            out_ref,
            kbuf, vbuf, wqa_buf, wqb_buf, woa_buf, wob_buf, x_buf, gw_buf,
            q_tab, ga_tab, gb_tab, acc_ref,
            k_sem, v_sem, w_sem, s_sem):

    def slot_of(t):
        return t % NS if isinstance(t, int) else lax.rem(t, NS)

    def step_base(t):
        return (t // SPU) * (NSTR * S) + (t % SPU) * G

    def kv_copy(src, base, buf, sem, slot, i, a):
        row = base + (i * S + a * R)
        if not isinstance(row, int):
            row = pl.multiple_of(row, R)
        return pltpu.make_async_copy(src.at[pl.ds(row, R), :],
                                     buf.at[slot, pl.ds(i * G + a * R, R), :], sem)

    def part_of(lst, part, nparts):
        n = len(lst) // nparts
        return list(enumerate(lst))[part * n:(part + 1) * n]

    def start_pair(k_src, kt, v_src, vt, gstep, part=0, nparts=1):
        kslot, vslot = slot_of(gstep), slot_of(gstep - 1)
        kb_, vb_ = step_base(kt), step_base(vt)
        for _, (i, a) in part_of(RR, part, nparts):
            kv_copy(k_src, kb_, kbuf, k_sem.at[kslot], kslot, i, a).start(priority=0)
            kv_copy(v_src, vb_, vbuf, v_sem.at[vslot], vslot, i, a).start(priority=1)

    def start_k_alone(src, t, slot):
        base = step_base(t)
        for n, (i, a) in enumerate(RR):
            kv_copy(src, base, kbuf, k_sem.at[slot], slot, i, a).start(priority=n % 2)

    def wait_k(slot):
        pltpu.make_async_copy(kbuf.at[slot], kbuf.at[slot], k_sem.at[slot]).wait()

    def wait_v(slot):
        pltpu.make_async_copy(vbuf.at[slot], vbuf.at[slot], v_sem.at[slot]).wait()

    def start_w_pair(wq_src, wq_dst, wq_sem, wo_src, wo_dst, wo_sem, n):
        p = (n % 4) * (NW // 4) + n // 4
        r = (p // 4) * 16
        c = (p % 4) * 1024
        ro = p * 32
        if not isinstance(n, int):
            r = pl.multiple_of(r, 16)
            c = pl.multiple_of(c, 1024)
            ro = pl.multiple_of(ro, 32)
        pltpu.make_async_copy(wq_src.at[pl.ds(r, 16), pl.ds(c, 1024)],
                              wq_dst.at[pl.ds(r, 16), pl.ds(c, 1024)], wq_sem).start(priority=0)
        pltpu.make_async_copy(wo_src.at[pl.ds(ro, 32), :],
                              wo_dst.at[pl.ds(ro, 32), :], wo_sem).start(priority=1)

    def wait_all(buf, sem):
        pltpu.make_async_copy(buf, buf, sem).wait()

    cx = pltpu.make_async_copy(x_hbm, x_buf, s_sem.at[0])
    cg = pltpu.make_async_copy(gw_hbm, gw_buf, s_sem.at[1])
    cx.start(priority=0)
    cg.start(priority=0)
    for n in range(NW):
        start_w_pair(wqb_hbm, wqb_buf, w_sem.at[0], wob_hbm, wob_buf, w_sem.at[1], n)
    start_k_alone(kb_hbm, 0, 0)
    for t in range(1, LB - 1):
        start_pair(kb_hbm, t, vb_hbm, t - 1, t)

    cx.wait()
    cg.wait()
    x = x_buf[...].astype(f32)
    gw = gw_buf[...].astype(f32).reshape(1, D)
    gate = jax.nn.sigmoid(jnp.sum(x * gw, axis=1, keepdims=True))
    x8 = jnp.concatenate([x, jnp.zeros((8 - NB, D), f32)], axis=0).astype(bf16)
    gate8 = jnp.concatenate([gate, jnp.zeros((8 - NB, 1), f32)], axis=0)
    ga_tab[...] = jnp.broadcast_to(gate8, (8, D))
    gb_tab[...] = jnp.broadcast_to(1.0 - gate8, (8, D))
    acc_ref[...] = jnp.zeros_like(acc_ref)

    row_d = lax.broadcasted_iota(jnp.int32, (8, D), 0)
    row_g = lax.broadcasted_iota(jnp.int32, (8, G), 0)
    row_h = lax.broadcasted_iota(jnp.int32, (8, DH), 0)

    def fill_q_tab(wq_buf, dup, issue):
        per = 4 if dup else 8
        hp = H // NFILL
        for k in range(NFILL):
            issue(k)
            q_p = jnp.dot(x8, wq_buf[:, k * hp * DH:(k + 1) * hp * DH], preferred_element_type=f32)
            for b in range(NB):
                for j in range(hp // per):
                    rows = [q_p[b:b + 1, (j * per + r) * DH:(j * per + r + 1) * DH] for r in range(per)]
                    if dup:
                        rows = rows + rows
                    q_tab[b * (H // per) + k * (hp // per) + j] = jnp.concatenate(rows, axis=0)

    def sel(vals, rows):
        key = rows % 4 if len(vals) == 4 else rows // 4
        out = vals[-1]
        for k in range(len(vals) - 2, -1, -1):
            out = jnp.where(key == k, vals[k], out)
        return out

    def scores(slot, qs, streams):
        wait_k(slot)
        out = []
        for q, st in zip(qs, streams):
            vals = [lax.dot_general(q, kbuf[slot, pl.ds(i * G, G), :], (((1,), (1,)), ((), ())),
                                    preferred_element_type=f32) for i in st]
            out.append(sel(vals, row_g))
        return out

    def softmax_update(sl, st):
        m, l, acc = st
        mx = sl[0]
        for s_ in sl[1:]:
            mx = jnp.maximum(mx, s_)
        m_new = jnp.maximum(m, jnp.max(mx, axis=1, keepdims=True))
        alpha = jnp.exp((m - m_new) * SCALE)
        l = alpha * l
        ps = []
        for s_ in sl:
            p = jnp.exp((s_ - m_new) * SCALE)
            for k in range(NC):
                l = l + p[:, k * DH:(k + 1) * DH]
            ps.append(p.astype(bf16))
        return ps, m_new, l, alpha * acc

    def step(t, qs, streams, state, issue):
        slot = slot_of(t)
        ss = scores(slot, qs, streams)
        issue()
        mid = [softmax_update([s_], st) for s_, st in zip(ss, state)]
        wait_v(slot)
        new = []
        for (ps, m, l, acc), st in zip(mid, streams):
            vals = [jnp.dot(ps[0], vbuf[slot, pl.ds(i * G, G), :], preferred_element_type=f32) for i in st]
            new.append((m, l, acc + sel(vals, row_h)))
        return new

    def init_state(n):
        return [(jnp.full((8, 1), NEG, f32), jnp.zeros((8, DH), f32), jnp.zeros((8, DH), f32))
                for _ in range(n)]

    def finish(st):
        m, l, acc = st
        return (acc / jnp.sum(l, axis=1, keepdims=True)).astype(bf16).astype(f32)

    def project(o, nrows, w):
        lhs = jnp.concatenate([jnp.broadcast_to(o[r:r + 1, :], (8, DH)) for r in range(nrows)], axis=1)
        return jnp.dot(lhs.astype(bf16), w, preferred_element_type=f32)

    def flat(state):
        return tuple(v for st in state for v in st)

    def unflat(vals):
        return [tuple(vals[3 * j:3 * j + 3]) for j in range(len(vals) // 3)]

    def unit_b(u, carry, last=False):
        b = u // 2
        half = u % 2
        qs = [q_tab[b * 4 + half * 2 + j].astype(bf16) for j in range(2)]

        def body(c, vals):
            t = u * SPU + c

            @pl.when(t < NW // WPS)
            def _():
                for r in range(WPS):
                    start_w_pair(wqa_hbm, wqa_buf, w_sem.at[2], woa_hbm, woa_buf, w_sem.at[3], t * WPS + r)

            def issue():
                ck = t + LB
                if not last:
                    start_pair(kb_hbm, ck, vb_hbm, ck - 1, ck)
                    return

                @pl.when(ck < NTB)
                def _():
                    start_pair(kb_hbm, ck, vb_hbm, ck - 1, ck)

                @pl.when(ck == NTB)
                def _():
                    start_pair(ka_hbm, 0, vb_hbm, NTB - 1, ck)

                @pl.when(ck > NTB)
                def _():
                    start_pair(ka_hbm, ck - NTB, va_hbm, ck - NTB - 1, ck)

            return flat(step(t, qs, [[0, 1], [2, 3]], unflat(vals), issue))

        st = unflat(lax.fori_loop(0, SPU, body, flat(init_state(2))))
        res = None
        for j in range(2):
            row0 = pl.multiple_of((half * 16 + j * 8) * DH, 8 * DH)
            r = project(finish(st[j]), 8, wob_buf[pl.ds(row0, 8 * DH), :])
            res = r if res is None else res + r
        acc_ref[...] += jnp.where(row_d == b, res * gb_tab[...], 0.0)
        return carry

    wait_all(wqb_buf, w_sem.at[0])
    fill_q_tab(wqb_buf, False,
               lambda k: start_pair(kb_hbm, LB - 1, vb_hbm, LB - 2, LB - 1, k, NFILL))
    wait_all(wob_buf, w_sem.at[1])
    lax.fori_loop(0, NUB - 1, unit_b, 0)
    unit_b(NUB - 1, 0, last=True)

    wait_all(wqa_buf, w_sem.at[2])
    fill_q_tab(wqa_buf, True,
               lambda k: start_pair(ka_hbm, LB, va_hbm, LB - 1, NTB + LB, k, NFILL))
    wait_all(woa_buf, w_sem.at[3])

    a_streams = [[0, 1, 2, 3]]

    def body_a(u, qs, c, vals, issue=None):
        ta = u * SPU + c
        if issue is None:
            def issue():
                ck = ta + LA
                start_pair(ka_hbm, ck, va_hbm, ck - 1, NTB + ck)
        return flat(step(NTB + ta, qs, a_streams, unflat(vals), issue))

    def unit_a(u, carry):
        b = u // 8
        hq = u % 8
        qs = [q_tab[u].astype(bf16)]
        vals = lax.fori_loop(0, SPU, functools.partial(body_a, u, qs), flat(init_state(1)))
        row0 = pl.multiple_of(hq * 4 * DH, 4 * DH)
        res = project(finish(unflat(vals)[0]), 4, woa_buf[pl.ds(row0, 4 * DH), :])
        acc_ref[...] += jnp.where(row_d == b, res * ga_tab[...], 0.0)
        return carry

    lax.fori_loop(0, NUA - 1, unit_a, 0)

    u = NUA - 1
    qs = [q_tab[u].astype(bf16)]
    s0, s1 = slot_of(NTB + NTA - 2), slot_of(NTB + NTA - 1)

    def issue_last_v():
        base = step_base(NTA - 1)
        for i, a in RR:
            kv_copy(va_hbm, base, vbuf, v_sem.at[s1], s1, i, a).start(priority=1)

    vals = lax.fori_loop(0, SPU - LA, functools.partial(body_a, u, qs), flat(init_state(1)))
    vals = body_a(u, qs, SPU - LA, vals, issue=issue_last_v)
    vals = lax.fori_loop(SPU - LA + 1, SPU - 2,
                         functools.partial(body_a, u, qs, issue=lambda: None), vals)
    sa = scores(s0, qs, a_streams)[0]
    sb = scores(s1, qs, a_streams)[0]
    ps, m, l, acc = softmax_update([sa, sb], unflat(vals)[0])
    inv_l = 1.0 / jnp.sum(l, axis=1, keepdims=True)
    for c, slot in enumerate((s0, s1)):
        wait_v(slot)
        pv = [jnp.dot(ps[c], vbuf[slot, pl.ds(i * G, G), :], preferred_element_type=f32)
              for i in range(NSTR)]
        acc = acc + sel(pv, row_h)
    o = (acc * inv_l).astype(bf16).astype(f32)
    res = project(o, 4, woa_buf[pl.ds((u % 8) * 4 * DH, 4 * DH), :])
    final = acc_ref[...] + jnp.where(row_d == u // 8, res * ga_tab[...], 0.0)
    out_ref[...] = final[0:NB, :].astype(out_ref.dtype)


_SCRATCH = [
    pltpu.VMEM((NS, CH, DH), bf16),
    pltpu.VMEM((NS, CH, DH), bf16),
    pltpu.VMEM((D, H * DH), bf16),
    pltpu.VMEM((D, H * DH), bf16),
    pltpu.VMEM((H * DH, D), bf16),
    pltpu.VMEM((H * DH, D), bf16),
    pltpu.VMEM((NB, D), bf16),
    pltpu.VMEM((D,), bf16),
    pltpu.VMEM((NUA, 8, DH), f32),
    pltpu.VMEM((8, D), f32),
    pltpu.VMEM((8, D), f32),
    pltpu.VMEM((8, D), f32),
    pltpu.SemaphoreType.DMA((NS,)),
    pltpu.SemaphoreType.DMA((NS,)),
    pltpu.SemaphoreType.DMA((4,)),
    pltpu.SemaphoreType.DMA((2,)),
]


@jax.jit
def pallas_gated_mix__mha_block_cached__gqa_block_cached__decode_kernel(
    A_x, A_k_cache, A_v_cache, A_wq, A_wo, B_x, B_k_cache, B_v_cache, B_wq, B_wo, gate_w,
):
    del B_x
    ka = A_k_cache.reshape(NB * H * S, DH)
    va = A_v_cache.reshape(NB * H * S, DH)
    kb = B_k_cache.reshape(NB * HKV * S, DH)
    vb = B_v_cache.reshape(NB * HKV * S, DH)
    any_spec = pl.BlockSpec(memory_space=pl.ANY)
    out = pl.pallas_call(
        _kernel,
        out_shape=jax.ShapeDtypeStruct((NB, D), bf16),
        in_specs=[any_spec] * 10,
        out_specs=pl.BlockSpec(memory_space=pltpu.VMEM),
        scratch_shapes=_SCRATCH,
        compiler_params=pltpu.CompilerParams(vmem_limit_bytes=64 * 1024 * 1024,
                                             disable_bounds_checks=True,
                                             disable_semaphore_checks=True),
    )(A_x.reshape(NB, D), ka, va, A_wq, A_wo, kb, vb, B_wq, B_wo, gate_w)
    return out.reshape(NB, 1, D)
```
